```python
import jax
import jax.numpy as jnp

def _softmax(x, axis=-1):
    return jax.nn.softmax(x, axis=axis)

def _gelu(x):
    return jax.nn.gelu(x, approximate=True)

def _silu(x):
    return jax.nn.silu(x)

def _sigmoid(x):
    return jax.nn.sigmoid(x)

def _layernorm(x, axis=-1, eps=1e-05):
    m = jnp.mean(x, axis=axis, keepdims=True)
    v = jnp.var(x, axis=axis, keepdims=True)
    return (x - m) / jnp.sqrt(v + eps)

def _scatter_add(tgt, idx, src, axis=0):
    return tgt.at[idx].add(src)

def _segment_sum(src, seg, n):
    return jax.ops.segment_sum(src, seg, n)

class _Rng:

    def __init__(self, key):
        self._k = key

    def _next(self):
        self._k, sub = jax.random.split(self._k)
        return sub

    def normal(self, shape):
        return jax.random.normal(self._next(), shape, dtype=jnp.bfloat16)

    def randint(self, lo, hi, shape):
        return jax.random.randint(self._next(), shape, lo, hi, dtype=jnp.int32)

    def uniform(self, shape, lo=0.0, hi=1.0):
        return jax.random.uniform(self._next(), shape, jnp.bfloat16, lo, hi)

    def permutation(self, n):
        return jax.random.permutation(self._next(), n)
kernel_name = 'concat_heads__sliding_local_dilated__memory_aug_recurrent_mem_tr__prompt'

def setup_inputs():
    _rng = _Rng(jax.random.key(int.from_bytes(__import__("os").urandom(4), "little")))
    _w = lambda a: (lambda t: t.astype(jnp.bfloat16) if jnp.issubdtype(t.dtype, jnp.floating) else t)(jnp.asarray(a))

    def _A_setup():
        B, S, D = (1, 2048, 640)
        return {'x': _w((lambda *s: _rng.normal(s) * 0.05)(B, S, D)), 'wqkv': _w((lambda *s: _rng.normal(s) * 0.05)(D, 3 * D)), 'wo': _w((lambda *s: _rng.normal(s) * 0.05)(D, D))}
    _A_in = _A_setup()

    def _B_setup():
        B, S, Dm = (1, 2048, 640)
        H, Dh = (32, 192)
        M, seg = (8, 32)
        seg = min(seg, S)
        S = S // seg * seg
        return {'x': _w((lambda *s: _rng.normal(s) * 0.05)(B, S, Dm)), 'mem0': _w((lambda *s: _rng.normal(s) * 0.05)(B, M, Dm)), 'Wq': _w((lambda *s: _rng.normal(s) * 0.05)(Dm, H, Dh) * Dm ** (-0.5)), 'Wk': _w((lambda *s: _rng.normal(s) * 0.05)(Dm, H, Dh) * Dm ** (-0.5)), 'Wv': _w((lambda *s: _rng.normal(s) * 0.05)(Dm, H, Dh) * Dm ** (-0.5)), 'Wo': _w((lambda *s: _rng.normal(s) * 0.05)(H, Dh, Dm) * (H * Dh) ** (-0.5)), 'seg_len': seg}
    _B_in = _B_setup()
    return {'A_x': _A_in['x'], 'A_wqkv': _A_in['wqkv'], 'A_wo': _A_in['wo'], 'B_x': _B_in['x'], 'B_mem0': _B_in['mem0'], 'B_Wq': _B_in['Wq'], 'B_Wk': _B_in['Wk'], 'B_Wv': _B_in['Wv'], 'B_Wo': _B_in['Wo'], 'B_seg_len': _B_in['seg_len']}

def reference(A_x, A_wqkv, A_wo, B_x, B_mem0, B_Wq, B_Wk, B_Wv, B_Wo, B_seg_len):

    def _A_ref(x, wqkv, wo):
        B, S, D = x.shape
        H = 32
        Dh = D // H
        W, dil = (8, 2)
        qkv = (lambda x, *d: x.transpose(*d))((x @ wqkv).reshape(B, S, 3, H, Dh), 2, 0, 3, 1, 4)
        q, k, v = (qkv[0], qkv[1], qkv[2])
        scale = Dh ** (-0.5)
        pos = jnp.arange(S)
        off = jnp.arange(W) * dil
        idx = pos[:, None] - off[None, :]
        mask = idx >= 0
        idx_c = jnp.where(mask, idx, 0).reshape(-1)
        kg = k[:, :, idx_c, :].reshape(B, H, S, W, Dh)
        vg = v[:, :, idx_c, :].reshape(B, H, S, W, Dh)
        logits = jnp.einsum('bhsd,bhswd->bhsw', q, kg) * scale
        logits = jnp.where(mask[None, None, :, :], logits, -1000000000.0)
        attn = _softmax(logits, axis=-1)
        o = jnp.einsum('bhsw,bhswd->bhsd', attn, vg)
        return (lambda x, *d: x.transpose(*d))(o, 0, 2, 1, 3).reshape(B, S, D) @ wo

    def _B_ref(x, mem0, Wq, Wk, Wv, Wo, seg_len):
        B, S, Dm = x.shape
        H, Dh = (Wq.shape[1], Wq.shape[2])
        M = mem0.shape[1]
        scale = Dh ** (-0.5)
        n_seg = S // seg_len
        L = M + seg_len
        idx = jnp.arange(L)
        mask = (idx[:, None] < M) | (idx[:, None] >= idx[None, :])
        mem = mem0
        outs = []
        for s in range(n_seg):
            xs = x[:, s * seg_len:(s + 1) * seg_len, :].copy()
            h = jnp.concatenate([mem, xs], axis=1)
            q = jnp.einsum('btd,dhe->bhte', h, Wq)
            k = jnp.einsum('btd,dhe->bhte', h, Wk)
            v = jnp.einsum('btd,dhe->bhte', h, Wv)
            scores = jnp.einsum('bhqe,bhke->bhqk', q, k) * scale
            scores = jnp.where(mask[None, None], scores, -1000000000.0)
            p = _softmax(scores, axis=-1)
            o = jnp.einsum('bhqk,bhke->bhqe', p, v)
            o = jnp.einsum('bhte,hed->btd', o, Wo)
            mem = o[:, :M, :].copy()
            outs.append(o[:, M:, :])
        return jnp.concatenate(outs, axis=1)
    a = _A_ref(A_x, A_wqkv, A_wo)
    b = _B_ref(B_x, B_mem0, B_Wq, B_Wk, B_Wv, B_Wo, B_seg_len)
    return jnp.concatenate([a, b], axis=-1)
```

```python
import functools

import jax
import jax.numpy as jnp
from jax import lax
import jax.experimental.pallas as pl
import jax.experimental.pallas.tpu as pltpu

BF16 = jnp.bfloat16
F32 = jnp.float32
U32 = jnp.uint32
LANES = 128

_NN = (((1,), (0,)), ((), ()))
_NT = (((1,), (1,)), ((), ()))

A_HEADS = 32
A_WIN = 8
A_DIL = 2
A_HALO = 16
A_CHUNK = 256
A_SUB = 16
MASK_VALUE = -1000000000.0

D_QK, D_PV, D_WO = 1, 3, 6


def _dot(a, b, dims=_NN):
    return lax.dot_general(a, b, dims, preferred_element_type=F32)


def _kernel(
    ax_hbm, awqkv_hbm, awo_hbm, bx_hbm, mem_hbm, wq_hbm, wk_hbm, wv_hbm, wo_hbm,
    out_hbm,
    ax_v, awqkv_v, awo_v, awqkv_p, awo_p, ak_v, av_v, aout_v,
    bx_v, mem_v, wt_v, wqkv_v, wo_v, h_v, bout_v,
    sem_a, sem_ax, sem_w, sem_b, sem_out,
    *, seg, b_heads, b_dh,
):
    S, D = ax_hbm.shape
    n_t = D // LANES
    a_dh = D // A_HEADS
    n_chunk = S // A_CHUNK
    M = mem_hbm.shape[0]
    L = seg + M
    n_seg = S // seg
    n_pair = b_heads // 2
    PW = 2 * b_dh
    w_hbm = (wq_hbm, wk_hbm, wv_hbm)

    cp_awqkv = pltpu.make_async_copy(awqkv_hbm, awqkv_v, sem_a.at[0])
    cp_awo = pltpu.make_async_copy(awo_hbm, awo_v, sem_a.at[1])

    def cp_ax(c):
        rows = pl.ds(pl.multiple_of(c * A_CHUNK, A_CHUNK), A_CHUNK)
        return pltpu.make_async_copy(ax_hbm.at[rows], ax_v.at[rows], sem_ax.at[c])

    ppg = n_pair // n_chunk
    grows = ppg * PW

    def cp_w(g, m):
        rows = pl.ds(pl.multiple_of(g * grows, grows), grows)
        return pltpu.make_async_copy(w_hbm[m].at[rows], wt_v.at[m, rows], sem_w.at[3 * g + m])

    def cp_wo(t):
        return pltpu.make_async_copy(
            wo_hbm.at[:, pl.ds(t * LANES, LANES)], wo_v.at[t], sem_b.at[t])

    cp_bx = pltpu.make_async_copy(bx_hbm, bx_v, sem_b.at[n_t])
    cp_mem = pltpu.make_async_copy(mem_hbm, mem_v, sem_b.at[n_t + 1])

    cp_awqkv.start()
    cp_awo.start()
    cp_ax(0).start()
    for g in range(n_chunk):
        for m in range(3):
            cp_w(g, m).start()
        if g + 1 < n_chunk:
            cp_ax(g + 1).start()
    cp_mem.start()
    cp_bx.start()
    for t in range(n_t):
        cp_wo(t).start()

    r_i = lax.broadcasted_iota(jnp.int32, (D, D), 0)
    c_i = lax.broadcasted_iota(jnp.int32, (D, D), 1)
    perm = (r_i == (c_i % A_HEADS) * a_dh + c_i // A_HEADS).astype(F32).astype(BF16)
    perm_t = (c_i == (r_i % A_HEADS) * a_dh + r_i // A_HEADS).astype(F32).astype(BF16)
    cp_awqkv.wait()
    for m in range(3):
        cols = slice(m * D, (m + 1) * D)
        awqkv_p[:, cols] = _dot(awqkv_v[:, cols], perm).astype(BF16)
    cp_awo.wait()
    awo_p[...] = _dot(perm_t, awo_v[...]).astype(BF16)

    a_scale = float(a_dh) ** -0.5

    def a_chunk(c, carry):
        r0 = pl.multiple_of(c * A_CHUNK, A_CHUNK)
        cp_ax(c).wait()
        for m in range(3):
            cp_w(c, m).wait()

        x = ax_v[pl.ds(r0, A_CHUNK), :]
        k = _dot(x, awqkv_p[:, D:2 * D])
        for t in range(n_t):
            ak_v[t, pl.ds(r0 + A_HALO, A_CHUNK), :] = k[:, t * LANES:(t + 1) * LANES]
        v = _dot(x, awqkv_p[:, 2 * D:3 * D])
        for t in range(n_t):
            av_v[t, pl.ds(r0 + A_HALO, A_CHUNK), :] = v[:, t * LANES:(t + 1) * LANES]

        @pl.when(c == 0)
        def _():
            for t in range(n_t):
                cols = slice(t * LANES, (t + 1) * LANES)
                ak_v[t, 0:A_HALO, :] = jnp.broadcast_to(k[0:1, cols], (A_HALO, LANES))
                av_v[t, 0:A_HALO, :] = jnp.broadcast_to(v[0:1, cols], (A_HALO, LANES))

        q = _dot(x, awqkv_p[:, 0:D])
        o_blocks = []
        for b in range(A_CHUNK // A_SUB):
            rb = b * A_SUB
            pos = r0 + rb + lax.broadcasted_iota(jnp.int32, (A_SUB, LANES), 0)
            logits = []
            for w in range(A_WIN):
                rows = pl.ds(r0 + (A_HALO + rb - w * A_DIL), A_SUB)
                acc = None
                for t in range(n_t):
                    term = q[rb:rb + A_SUB, t * LANES:(t + 1) * LANES] * ak_v[t, rows, :]
                    acc = term if acc is None else acc + term
                acc = acc + pltpu.roll(acc, 2 * A_HEADS, axis=1)
                acc = acc + pltpu.roll(acc, A_HEADS, axis=1)
                lg = acc * a_scale
                if w > 0 and rb < w * A_DIL:
                    lg = jnp.where(pos >= w * A_DIL, lg, MASK_VALUE)
                logits.append(lg)
            mx = functools.reduce(jnp.maximum, logits)
            es = [jnp.exp(lg - mx) for lg in logits]
            inv = 1.0 / functools.reduce(jnp.add, es)
            o_t = []
            for t in range(n_t):
                acc = None
                for w in range(A_WIN):
                    rows = pl.ds(r0 + (A_HALO + rb - w * A_DIL), A_SUB)
                    term = es[w] * av_v[t, rows, :]
                    acc = term if acc is None else acc + term
                o_t.append((acc * inv).astype(BF16))
            o_blocks.append(jnp.concatenate(o_t, axis=1))
        o = jnp.concatenate(o_blocks, axis=0)
        aout_v[pl.ds(r0, A_CHUNK), :] = _dot(o, awo_p[...]).astype(BF16)

        for j in range(ppg):
            pair = c * ppg + j
            rows = pl.ds(pl.multiple_of(pair * PW, PW), PW)
            for m in range(3):
                wqkv_v[pair, :, m * PW:(m + 1) * PW] = pltpu.bitcast(wt_v[m, rows, :].T, U32)
        return carry

    lax.fori_loop(0, n_chunk, a_chunk, 0)

    cp_mem.wait()
    cp_bx.wait()
    for t in range(n_t):
        cp_wo(t).wait()

    cp_aout = pltpu.make_async_copy(aout_v, out_hbm.at[:, pl.ds(0, D)], sem_out.at[0])
    cp_aout.start()

    b_scale = float(b_dh) ** -0.5
    wo_w = wo_v.bitcast(U32)
    h_v[seg:L, :] = mem_v[...].astype(F32)

    def b_step(s, carry):
        r0 = pl.multiple_of(s * seg, seg)
        h_v[0:seg, :] = bx_v[pl.ds(r0, seg), :].astype(F32)

        row = lax.broadcasted_iota(jnp.int32, (L, 2 * L), 0)
        col = lax.broadcasted_iota(jnp.int32, (L, 2 * L), 1)
        first = col < L
        key = jnp.where(first, col, col - L)
        mask = (row >= seg) | (key >= seg) | (key <= row)
        lo = lax.broadcasted_iota(jnp.int32, (L, LANES), 1) < b_dh - LANES

        def block_diag(t):
            z = jnp.zeros((L, LANES), F32)
            mid = t[:, LANES:2 * LANES]
            top = jnp.concatenate([t[:, 0:LANES], jnp.where(lo, mid, 0.0), z], axis=1)
            bot = jnp.concatenate([z, jnp.where(lo, 0.0, mid), t[:, 2 * LANES:]], axis=1)
            return jnp.concatenate([top, bot], axis=0).astype(BF16)

        q, kk, vv, p, o = {}, {}, {}, {}, {}
        acc = [None]

        def project(i):
            h = h_v[...]
            w = pltpu.bitcast(wqkv_v[i], BF16)
            kk[i] = block_diag(_dot(h, w[:, PW:2 * PW]))
            q[i] = _dot(h, w[:, 0:PW])
            vv[i] = block_diag(_dot(h, w[:, 2 * PW:3 * PW]))

        def scores(i):
            sc = _dot(q.pop(i), kk.pop(i), _NT) * b_scale
            sc = jnp.where(mask, sc, MASK_VALUE)
            m0 = jnp.max(jnp.where(first, sc, -jnp.inf), axis=1, keepdims=True)
            m1 = jnp.max(jnp.where(first, -jnp.inf, sc), axis=1, keepdims=True)
            e = jnp.exp(sc - jnp.where(first, m0, m1))
            s0 = jnp.sum(jnp.where(first, e, 0.0), axis=1, keepdims=True)
            s1 = jnp.sum(jnp.where(first, 0.0, e), axis=1, keepdims=True)
            p[i] = e / jnp.where(first, s0, s1)

        def values(i):
            o[i] = _dot(p.pop(i), vv.pop(i))

        def out_proj(i):
            rows = slice(i * PW // 2, (i + 1) * PW // 2)
            w = jnp.concatenate(
                [pltpu.bitcast(wo_w[t, rows, :], BF16) for t in range(n_t)], axis=1)
            r = _dot(o.pop(i), w)
            acc[0] = r if acc[0] is None else acc[0] + r

        done = 0
        i = 0
        while done < n_pair:
            if i < n_pair:
                project(i)
            if 0 <= i - D_QK < n_pair:
                scores(i - D_QK)
            if 0 <= i - D_PV < n_pair:
                values(i - D_PV)
            if i < n_pair:
                n = 1 if i >= D_WO else 0
            else:
                left = n_pair + D_PV - i
                ready = min(n_pair, i - D_PV) - done
                n = min(-(-(n_pair - 1 - done) // left), ready) if left > 0 else n_pair - done
            for _ in range(n):
                out_proj(done)
                done += 1
            i += 1

        res = acc[0].astype(BF16)
        bout_v[pl.ds(r0, seg), :] = res[0:seg]
        h_v[seg:L, :] = res[seg:L].astype(F32)
        return carry

    n_blk = 8
    blk = n_seg // n_blk

    def b_block(j, carry):
        lax.fori_loop(j * blk, (j + 1) * blk, b_step, 0)
        rows = pl.ds(pl.multiple_of(j * (blk * seg), blk * seg), blk * seg)
        pltpu.make_async_copy(
            bout_v.at[rows], out_hbm.at[rows, pl.ds(D, D)], sem_out.at[1]).start()
        return carry

    lax.fori_loop(0, n_blk, b_block, 0)

    cp_aout.wait()
    pltpu.make_async_copy(bout_v, out_hbm.at[:, pl.ds(D, D)], sem_out.at[1]).wait()


@functools.partial(jax.jit, static_argnames=("B_seg_len",))
def pallas_concat_heads__sliding_local_dilated__memory_aug_recurrent_mem_tr__prompt_kernel(
    A_x: jax.Array,
    A_wqkv: jax.Array,
    A_wo: jax.Array,
    B_x: jax.Array,
    B_mem0: jax.Array,
    B_Wq: jax.Array,
    B_Wk: jax.Array,
    B_Wv: jax.Array,
    B_Wo: jax.Array,
    B_seg_len: int,
):
    B, S, D = A_x.shape
    M = B_mem0.shape[1]
    _, H, Dh = B_Wq.shape
    seg = int(B_seg_len)
    assert B == 1 and B_x.shape == (B, S, D) and S % A_CHUNK == 0 and S % (8 * seg) == 0
    assert D % LANES == 0 and D % A_HEADS == 0 and 4 * A_HEADS == LANES
    assert 2 * Dh == 3 * LANES and 2 * (seg + M) <= LANES and seg % 16 == 0 and M % 8 == 0
    n_t = D // LANES
    n_chunk = S // A_CHUNK
    assert (H // 2) % n_chunk == 0

    def head_major(w):
        return jnp.transpose(w, (1, 2, 0)).reshape(H * Dh, D)

    any_spec = pl.BlockSpec(memory_space=pl.ANY)
    out = pl.pallas_call(
        functools.partial(_kernel, seg=seg, b_heads=H, b_dh=Dh),
        in_specs=[any_spec] * 9,
        out_specs=any_spec,
        out_shape=jax.ShapeDtypeStruct((S, 2 * D), BF16),
        scratch_shapes=[
            pltpu.VMEM((S, D), BF16),
            pltpu.VMEM((D, 3 * D), BF16),
            pltpu.VMEM((D, D), BF16),
            pltpu.VMEM((D, 3 * D), BF16),
            pltpu.VMEM((D, D), BF16),
            pltpu.VMEM((n_t, A_HALO + S, LANES), F32),
            pltpu.VMEM((n_t, A_HALO + S, LANES), F32),
            pltpu.VMEM((S, D), BF16),
            pltpu.VMEM((S, D), BF16),
            pltpu.VMEM((M, D), BF16),
            pltpu.VMEM((3, H * Dh, D), BF16),
            pltpu.VMEM((H // 2, D // 2, 6 * Dh), U32),
            pltpu.VMEM((n_t, H * Dh, LANES), BF16),
            pltpu.VMEM((seg + M, D), F32),
            pltpu.VMEM((S, D), BF16),
            pltpu.SemaphoreType.DMA((2,)),
            pltpu.SemaphoreType.DMA((n_chunk,)),
            pltpu.SemaphoreType.DMA((3 * n_chunk,)),
            pltpu.SemaphoreType.DMA((n_t + 2,)),
            pltpu.SemaphoreType.DMA((2,)),
        ],
        compiler_params=pltpu.CompilerParams(vmem_limit_bytes=112 * 1024 * 1024),
        name="mbkern",
    )(
        A_x.reshape(S, D),
        A_wqkv,
        A_wo,
        B_x.reshape(S, D),
        B_mem0.reshape(M, D),
        head_major(B_Wq),
        head_major(B_Wk),
        head_major(B_Wv),
        B_Wo.reshape(H * Dh, D),
    )
    return out.reshape(B, S, 2 * D)
```

```python
import functools

import jax
import jax.numpy as jnp
from jax import lax
import jax.experimental.pallas as pl
import jax.experimental.pallas.tpu as pltpu

BF16 = jnp.bfloat16
F32 = jnp.float32
U32 = jnp.uint32
LANES = 128

_NN = (((1,), (0,)), ((), ()))
_NT = (((1,), (1,)), ((), ()))

A_HEADS = 32
A_WIN = 8
A_DIL = 2
A_HALO = 16
A_CHUNK = 256
A_ROWS = 64
A_D_OUT = 2
A_SUB = 16
MASK_VALUE = -1000000000.0

D_QK, D_PV, D_WO = 1, 3, 6


def _dot(a, b, dims=_NN):
    return lax.dot_general(a, b, dims, preferred_element_type=F32)


def _kernel(
    ax_hbm, awqkv_hbm, awo_hbm, bx_hbm, mem_hbm, wq_hbm, wk_hbm, wv_hbm, wo_hbm,
    out_hbm,
    ax_v, awqkv_v, awo_v, awqkv_p, awo_p, atmp_v, ak_v, av_v, aout_v,
    bx_v, mem_v, wt_v, wqkv_v, wo_v, h_v, bout_v,
    sem_in, sem_out,
    *, seg, b_heads, b_dh,
):
    S, D = ax_hbm.shape
    n_t = D // LANES
    a_dh = D // A_HEADS
    n_chunk = S // A_CHUNK
    M = mem_hbm.shape[0]
    L = seg + M
    n_seg = S // seg
    n_pair = b_heads // 2
    PW = 2 * b_dh
    w_hbm = (wq_hbm, wk_hbm, wv_hbm, wo_hbm)

    def qkv_cols(j):
        return pl.ds(pl.multiple_of(((j + 1) % 3) * D, LANES), D)

    def cp_awqkv(j):
        return pltpu.make_async_copy(awqkv_hbm.at[:, qkv_cols(j)], awqkv_v.at[j], sem_in.at[j])

    cp_awo = pltpu.make_async_copy(awo_hbm, awo_v, sem_in.at[3])
    cp_mem = pltpu.make_async_copy(mem_hbm, mem_v, sem_in.at[4])

    def chunk_rows(c):
        return pl.ds(pl.multiple_of(c * A_CHUNK, A_CHUNK), A_CHUNK)

    def cp_ax(c):
        return pltpu.make_async_copy(
            ax_hbm.at[chunk_rows(c)], ax_v.at[chunk_rows(c)], sem_in.at[5 + c])

    def cp_bx(c):
        return pltpu.make_async_copy(
            bx_hbm.at[chunk_rows(c)], bx_v.at[chunk_rows(c)], sem_in.at[5 + n_chunk + c])

    ppg = n_pair // n_chunk
    grows = ppg * PW

    def cp_w(g, m):
        rows = pl.ds(pl.multiple_of(g * grows, grows), grows)
        return pltpu.make_async_copy(
            w_hbm[m].at[rows], wt_v.at[m, rows], sem_in.at[5 + (2 + m) * n_chunk + g])

    for j in range(3):
        cp_awqkv(j).start()
    cp_ax(0).start()
    cp_awo.start()
    for g in range(n_chunk):
        for m in range(3):
            cp_w(g, m).start()
        if g + 1 < n_chunk:
            cp_ax(g + 1).start()
    cp_mem.start()
    cp_bx(0).start()
    for g in range(n_chunk):
        cp_w(g, 3).start()
    for c in range(1, n_chunk):
        cp_bx(c).start()

    def regroup_rows(w):
        for t in range(n_t):
            atmp_v[t] = w[:, t * LANES:(t + 1) * LANES]
        return jnp.concatenate([
            jnp.concatenate(
                [atmp_v[t, pl.ds(d, A_HEADS, stride=a_dh), :] for t in range(n_t)], axis=1
            ).astype(BF16)
            for d in range(a_dh)
        ], axis=0)

    def regroup_qkv(j, carry):
        cp_awqkv(j).wait()
        awqkv_p[j] = pltpu.bitcast(regroup_rows(awqkv_v[j].astype(F32).T).T, U32)
        return carry

    lax.fori_loop(0, 3, regroup_qkv, 0)
    cp_awo.wait()
    awo_p[...] = pltpu.bitcast(regroup_rows(awo_v[...].astype(F32)), U32)

    cp_ax(0).wait()
    v0 = _dot(ax_v[0:16, :], pltpu.bitcast(awqkv_p[1], BF16))
    for t in range(n_t):
        ak_v[t, 0:A_HALO, :] = jnp.zeros((A_HALO, LANES), F32)
        av_v[t, 0:A_HALO, :] = jnp.broadcast_to(
            v0[0:1, t * LANES:(t + 1) * LANES], (A_HALO, LANES))

    a_scale = float(a_dh) ** -0.5

    def a_chunk(c, carry):
        r0 = pl.multiple_of(c * A_CHUNK, A_CHUNK)

        @pl.when(c > 0)
        def _():
            cp_ax(c).wait()

        for m in range(3):
            cp_w(c, m).wait()

        qs, os = {}, {}

        def project(i):
            x = ax_v[pl.ds(r0 + i * A_ROWS, A_ROWS), :]
            rows = pl.ds(r0 + (A_HALO + i * A_ROWS), A_ROWS)
            for j, dst in enumerate((ak_v, av_v)):
                y = _dot(x, pltpu.bitcast(awqkv_p[j], BF16))
                for t in range(n_t):
                    dst[t, rows, :] = y[:, t * LANES:(t + 1) * LANES]
            qs[i] = _dot(x, pltpu.bitcast(awqkv_p[2], BF16))

        def attend(i):
            q = qs.pop(i)
            blocks = []
            for b in range(A_ROWS // A_SUB):
                rq = b * A_SUB
                rb = i * A_ROWS + rq
                logits = []
                for w in range(A_WIN):
                    rows = pl.ds(r0 + (A_HALO + rb - w * A_DIL), A_SUB)
                    acc = None
                    for t in range(n_t):
                        term = q[rq:rq + A_SUB, t * LANES:(t + 1) * LANES] * ak_v[t, rows, :]
                        acc = term if acc is None else acc + term
                    acc = acc + pltpu.roll(acc, 2 * A_HEADS, axis=1)
                    acc = acc + pltpu.roll(acc, A_HEADS, axis=1)
                    lg = acc * a_scale
                    if rb < w * A_DIL:
                        pos = r0 + rb + lax.broadcasted_iota(jnp.int32, (A_SUB, LANES), 0)
                        lg = jnp.where(pos >= w * A_DIL, lg, MASK_VALUE)
                    logits.append(lg)
                mx = functools.reduce(jnp.maximum, logits)
                es = [jnp.exp(lg - mx) for lg in logits]
                inv = 1.0 / functools.reduce(jnp.add, es)
                o_t = []
                for t in range(n_t):
                    acc = None
                    for w in range(A_WIN):
                        rows = pl.ds(r0 + (A_HALO + rb - w * A_DIL), A_SUB)
                        term = es[w] * av_v[t, rows, :]
                        acc = term if acc is None else acc + term
                    o_t.append((acc * inv).astype(BF16))
                blocks.append(jnp.concatenate(o_t, axis=1))
            os[i] = jnp.concatenate(blocks, axis=0)

        def out_proj(i):
            y = _dot(os.pop(i), pltpu.bitcast(awo_p[...], BF16))
            aout_v[pl.ds(r0 + i * A_ROWS, A_ROWS), :] = y.astype(BF16)

        def transpose_w(n):
            j, m = divmod(n, 3)
            pair = c * ppg + j
            rows = pl.ds(pl.multiple_of(pair * PW, PW), PW)
            wqkv_v[pair, :, m * PW:(m + 1) * PW] = pltpu.bitcast(wt_v[m, rows, :].T, U32)

        n_sub = A_CHUNK // A_ROWS
        n_tr = 3 * ppg
        for i in range(n_sub + A_D_OUT):
            if i < n_sub:
                project(i)
                for n in range(i * n_tr // n_sub, (i + 1) * n_tr // n_sub):
                    transpose_w(n)
            if 0 <= i - 1 < n_sub:
                attend(i - 1)
            if 0 <= i - A_D_OUT < n_sub:
                out_proj(i - A_D_OUT)
        return carry

    lax.fori_loop(0, n_chunk, a_chunk, 0)

    def repack_wo(g, carry):
        cp_w(g, 3).wait()
        rows = pl.ds(pl.multiple_of(g * grows, grows), grows)
        half = pl.ds(pl.multiple_of(g * (grows // 2), grows // 2), grows // 2)
        wo_v[half, :] = pltpu.bitcast(wt_v[3, rows, :], U32)
        return carry

    lax.fori_loop(0, n_chunk, repack_wo, 0)
    cp_mem.wait()

    cp_aout = pltpu.make_async_copy(aout_v, out_hbm.at[:, pl.ds(0, D)], sem_out.at[0])
    cp_aout.start()

    b_scale = float(b_dh) ** -0.5
    h_v[seg:L, :] = mem_v[...].astype(F32)

    def b_step(s, carry):
        r0 = pl.multiple_of(s * seg, seg)
        h_v[0:seg, :] = bx_v[pl.ds(r0, seg), :].astype(F32)

        row = lax.broadcasted_iota(jnp.int32, (L, 2 * L), 0)
        col = lax.broadcasted_iota(jnp.int32, (L, 2 * L), 1)
        first = col < L
        key = jnp.where(first, col, col - L)
        mask = (row >= seg) | (key >= seg) | (key <= row)
        lo = lax.broadcasted_iota(jnp.int32, (L, LANES), 1) < b_dh - LANES

        def block_diag(t):
            z = jnp.zeros((L, LANES), F32)
            mid = t[:, LANES:2 * LANES]
            top = jnp.concatenate([t[:, 0:LANES], jnp.where(lo, mid, 0.0), z], axis=1)
            bot = jnp.concatenate([z, jnp.where(lo, 0.0, mid), t[:, 2 * LANES:]], axis=1)
            return jnp.concatenate([top, bot], axis=0).astype(BF16)

        q, kk, vv, p, o = {}, {}, {}, {}, {}
        acc = [None]

        def project(i):
            h = h_v[...]
            w = pltpu.bitcast(wqkv_v[i], BF16)
            kk[i] = block_diag(_dot(h, w[:, PW:2 * PW]))
            q[i] = _dot(h, w[:, 0:PW])
            vv[i] = block_diag(_dot(h, w[:, 2 * PW:3 * PW]))

        def scores(i):
            sc = _dot(q.pop(i), kk.pop(i), _NT) * b_scale
            sc = jnp.where(mask, sc, MASK_VALUE)
            m0 = jnp.max(jnp.where(first, sc, -jnp.inf), axis=1, keepdims=True)
            m1 = jnp.max(jnp.where(first, -jnp.inf, sc), axis=1, keepdims=True)
            e = jnp.exp(sc - jnp.where(first, m0, m1))
            s0 = jnp.sum(jnp.where(first, e, 0.0), axis=1, keepdims=True)
            s1 = jnp.sum(jnp.where(first, 0.0, e), axis=1, keepdims=True)
            p[i] = e / jnp.where(first, s0, s1)

        def values(i):
            o[i] = _dot(p.pop(i), vv.pop(i))

        def out_proj(i):
            rows = slice(i * PW // 2, (i + 1) * PW // 2)
            r = _dot(o.pop(i), pltpu.bitcast(wo_v[rows, :], BF16))
            acc[0] = r if acc[0] is None else acc[0] + r

        done = 0
        i = 0
        while done < n_pair:
            if i < n_pair:
                project(i)
            if 0 <= i - D_QK < n_pair:
                scores(i - D_QK)
            if 0 <= i - D_PV < n_pair:
                values(i - D_PV)
            if i < n_pair:
                n = 1 if i >= D_WO else 0
            else:
                left = n_pair + D_PV - i
                ready = min(n_pair, i - D_PV) - done
                n = min(-(-(n_pair - 1 - done) // left), ready) if left > 0 else n_pair - done
            for _ in range(n):
                out_proj(done)
                done += 1
            i += 1

        res = acc[0].astype(BF16)
        bout_v[pl.ds(r0, seg), :] = res[0:seg]
        h_v[seg:L, :] = res[seg:L].astype(F32)
        return carry

    blk = n_seg // n_chunk

    def b_block(j, carry):
        cp_bx(j).wait()
        lax.fori_loop(j * blk, (j + 1) * blk, b_step, 0)
        rows = chunk_rows(j)
        pltpu.make_async_copy(
            bout_v.at[rows], out_hbm.at[rows, pl.ds(D, D)], sem_out.at[1]).start()
        return carry

    lax.fori_loop(0, n_chunk, b_block, 0)

    cp_aout.wait()
    pltpu.make_async_copy(bout_v, out_hbm.at[:, pl.ds(D, D)], sem_out.at[1]).wait()


@functools.partial(jax.jit, static_argnames=("B_seg_len",))
def pallas_concat_heads__sliding_local_dilated__memory_aug_recurrent_mem_tr__prompt_kernel(
    A_x: jax.Array,
    A_wqkv: jax.Array,
    A_wo: jax.Array,
    B_x: jax.Array,
    B_mem0: jax.Array,
    B_Wq: jax.Array,
    B_Wk: jax.Array,
    B_Wv: jax.Array,
    B_Wo: jax.Array,
    B_seg_len: int,
):
    B, S, D = A_x.shape
    M = B_mem0.shape[1]
    _, H, Dh = B_Wq.shape
    seg = int(B_seg_len)
    assert B == 1 and B_x.shape == (B, S, D) and S % A_CHUNK == 0 and A_CHUNK % seg == 0
    assert D % LANES == 0 and D % A_HEADS == 0 and 4 * A_HEADS == LANES
    assert 2 * Dh == 3 * LANES and 2 * (seg + M) <= LANES and seg % 16 == 0 and M % 8 == 0
    n_t = D // LANES
    n_chunk = S // A_CHUNK
    assert (H // 2) % n_chunk == 0

    def head_major(w):
        return jnp.transpose(w, (1, 2, 0)).reshape(H * Dh, D)

    any_spec = pl.BlockSpec(memory_space=pl.ANY)
    out = pl.pallas_call(
        functools.partial(_kernel, seg=seg, b_heads=H, b_dh=Dh),
        in_specs=[any_spec] * 9,
        out_specs=any_spec,
        out_shape=jax.ShapeDtypeStruct((S, 2 * D), BF16),
        scratch_shapes=[
            pltpu.VMEM((S, D), BF16),
            pltpu.VMEM((3, D, D), BF16),
            pltpu.VMEM((D, D), BF16),
            pltpu.VMEM((3, D // 2, D), U32),
            pltpu.VMEM((D // 2, D), U32),
            pltpu.VMEM((n_t, D, LANES), F32),
            pltpu.VMEM((n_t, A_HALO + S, LANES), F32),
            pltpu.VMEM((n_t, A_HALO + S, LANES), F32),
            pltpu.VMEM((S, D), BF16),
            pltpu.VMEM((S, D), BF16),
            pltpu.VMEM((M, D), BF16),
            pltpu.VMEM((4, H * Dh, D), BF16),
            pltpu.VMEM((H // 2, D // 2, 6 * Dh), U32),
            pltpu.VMEM((H * Dh // 2, D), U32),
            pltpu.VMEM((seg + M, D), F32),
            pltpu.VMEM((S, D), BF16),
            pltpu.SemaphoreType.DMA((5 + 6 * n_chunk,)),
            pltpu.SemaphoreType.DMA((2,)),
        ],
        compiler_params=pltpu.CompilerParams(vmem_limit_bytes=112 * 1024 * 1024),
        name="mbkern",
    )(
        A_x.reshape(S, D),
        A_wqkv,
        A_wo,
        B_x.reshape(S, D),
        B_mem0.reshape(M, D),
        head_major(B_Wq),
        head_major(B_Wk),
        head_major(B_Wv),
        B_Wo.reshape(H * Dh, D),
    )
    return out.reshape(B, S, 2 * D)
```

```python
import functools

import jax
import jax.numpy as jnp
from jax import lax
import jax.experimental.pallas as pl
import jax.experimental.pallas.tpu as pltpu

BF16 = jnp.bfloat16
F32 = jnp.float32
U32 = jnp.uint32
LANES = 128

_NN = (((1,), (0,)), ((), ()))
_NT = (((1,), (1,)), ((), ()))

A_HEADS = 32
A_WIN = 8
A_DIL = 2
A_HALO = 16
A_CHUNK = 256
A_ROWS = 64
A_D_OUT = 2
A_SUB = 16
MASK_VALUE = -1000000000.0

D_QK, D_PV, D_WO = 1, 3, 6
PRE = 8
FLAGS = None


def _dot(a, b, dims=_NN):
    return lax.dot_general(a, b, dims, preferred_element_type=F32)


def _kernel(
    ax_hbm, awqkv_hbm, awo_hbm, bx_hbm, mem_hbm, wq_hbm, wk_hbm, wv_hbm, wo_hbm,
    out_hbm,
    ax_v, awqkv_v, awo_v, awqkv_p, awo_p, atmp_v, ak_v, av_v, aout_v,
    bx_v, mem_v, wt_v, wqkv_v, wo_v, xpre_v, qpre_v, h_v, bout_v,
    sem_in, sem_out,
    *, seg, b_heads, b_dh,
):
    S, D = ax_hbm.shape
    n_t = D // LANES
    a_dh = D // A_HEADS
    n_chunk = S // A_CHUNK
    M = mem_hbm.shape[0]
    L = seg + M
    n_seg = S // seg
    n_pair = b_heads // 2
    PW = 2 * b_dh
    w_hbm = (wq_hbm, wk_hbm, wv_hbm, wo_hbm)

    def qkv_cols(j):
        return pl.ds(pl.multiple_of(((j + 1) % 3) * D, LANES), D)

    def cp_awqkv(j):
        return pltpu.make_async_copy(awqkv_hbm.at[:, qkv_cols(j)], awqkv_v.at[j], sem_in.at[j])

    cp_awo = pltpu.make_async_copy(awo_hbm, awo_v, sem_in.at[3])
    cp_mem = pltpu.make_async_copy(mem_hbm, mem_v, sem_in.at[4])

    def chunk_rows(c):
        return pl.ds(pl.multiple_of(c * A_CHUNK, A_CHUNK), A_CHUNK)

    def cp_ax(c):
        return pltpu.make_async_copy(
            ax_hbm.at[chunk_rows(c)], ax_v.at[chunk_rows(c)], sem_in.at[6 + c])

    cp_bx = pltpu.make_async_copy(bx_hbm, bx_v, sem_in.at[5])

    def pair_rows(i):
        return pl.ds(pl.multiple_of(i * PW, PW), PW)

    def cp_w(i, m):
        return pltpu.make_async_copy(
            w_hbm[m].at[pair_rows(i)], wt_v.at[m, pair_rows(i)],
            sem_in.at[6 + n_chunk + m * n_pair + i])

    for j in range(3):
        cp_awqkv(j).start()
    cp_ax(0).start()
    cp_awo.start()
    for c in range(1, n_chunk):
        cp_ax(c).start()
    cp_mem.start()
    cp_bx.start()

    def start_w(i, carry):
        for m in range(4):
            cp_w(i, m).start()
        return carry

    lax.fori_loop(0, n_pair, start_w, 0)

    def regroup_rows(w):
        for t in range(n_t):
            atmp_v[t] = w[:, t * LANES:(t + 1) * LANES]
        return jnp.concatenate([
            jnp.concatenate(
                [atmp_v[t, pl.ds(d, A_HEADS, stride=a_dh), :] for t in range(n_t)], axis=1
            ).astype(BF16)
            for d in range(a_dh)
        ], axis=0)

    def regroup_qkv(j, carry):
        cp_awqkv(j).wait()
        awqkv_p[j] = pltpu.bitcast(regroup_rows(awqkv_v[j].astype(F32).T).T, U32)
        return carry

    lax.fori_loop(0, 3, regroup_qkv, 0)
    cp_awo.wait()
    awo_p[...] = pltpu.bitcast(regroup_rows(awo_v[...].astype(F32)), U32)

    cp_ax(0).wait()
    v0 = _dot(ax_v[0:16, :], pltpu.bitcast(awqkv_p[1], BF16))
    for t in range(n_t):
        ak_v[t, 0:A_HALO, :] = jnp.zeros((A_HALO, LANES), F32)
        av_v[t, 0:A_HALO, :] = jnp.broadcast_to(
            v0[0:1, t * LANES:(t + 1) * LANES], (A_HALO, LANES))

    a_scale = float(a_dh) ** -0.5

    def a_chunk(c, carry):
        r0 = pl.multiple_of(c * A_CHUNK, A_CHUNK)

        @pl.when(c > 0)
        def _():
            cp_ax(c).wait()

        qs, os = {}, {}

        def project(i):
            x = ax_v[pl.ds(r0 + i * A_ROWS, A_ROWS), :]
            rows = pl.ds(r0 + (A_HALO + i * A_ROWS), A_ROWS)
            for j, dst in enumerate((ak_v, av_v)):
                y = _dot(x, pltpu.bitcast(awqkv_p[j], BF16))
                for t in range(n_t):
                    dst[t, rows, :] = y[:, t * LANES:(t + 1) * LANES]
            qs[i] = _dot(x, pltpu.bitcast(awqkv_p[2], BF16))

        def attend(i):
            q = qs.pop(i)
            blocks = []
            for b in range(A_ROWS // A_SUB):
                rq = b * A_SUB
                rb = i * A_ROWS + rq
                logits = []
                for w in range(A_WIN):
                    rows = pl.ds(r0 + (A_HALO + rb - w * A_DIL), A_SUB)
                    acc = None
                    for t in range(n_t):
                        term = q[rq:rq + A_SUB, t * LANES:(t + 1) * LANES] * ak_v[t, rows, :]
                        acc = term if acc is None else acc + term
                    acc = acc + pltpu.roll(acc, 2 * A_HEADS, axis=1)
                    acc = acc + pltpu.roll(acc, A_HEADS, axis=1)
                    lg = acc * a_scale
                    if rb < w * A_DIL:
                        pos = r0 + rb + lax.broadcasted_iota(jnp.int32, (A_SUB, LANES), 0)
                        lg = jnp.where(pos >= w * A_DIL, lg, MASK_VALUE)
                    logits.append(lg)
                mx = functools.reduce(jnp.maximum, logits)
                es = [jnp.exp(lg - mx) for lg in logits]
                inv = 1.0 / functools.reduce(jnp.add, es)
                o_t = []
                for t in range(n_t):
                    acc = None
                    for w in range(A_WIN):
                        rows = pl.ds(r0 + (A_HALO + rb - w * A_DIL), A_SUB)
                        term = es[w] * av_v[t, rows, :]
                        acc = term if acc is None else acc + term
                    o_t.append((acc * inv).astype(BF16))
                blocks.append(jnp.concatenate(o_t, axis=1))
            os[i] = jnp.concatenate(blocks, axis=0)

        def out_proj(i):
            y = _dot(os.pop(i), pltpu.bitcast(awo_p[...], BF16))
            aout_v[pl.ds(r0 + i * A_ROWS, A_ROWS), :] = y.astype(BF16)

        n_sub = A_CHUNK // A_ROWS
        for i in range(n_sub + A_D_OUT):
            if i < n_sub:
                project(i)
            if 0 <= i - 1 < n_sub:
                attend(i - 1)
            if 0 <= i - A_D_OUT < n_sub:
                out_proj(i - A_D_OUT)
        return carry

    lax.fori_loop(0, n_chunk, a_chunk, 0)

    cp_aout = pltpu.make_async_copy(aout_v, out_hbm.at[:, pl.ds(0, D)], sem_out.at[0])
    cp_aout.start()

    cp_mem.wait()
    cp_bx.wait()

    def gather_pre(s, carry):
        top = jnp.concatenate([
            bx_v[pl.ds(pl.multiple_of((2 * s + u) * seg, seg), 16), :].astype(F32)[0:PRE]
            for u in range(2)], axis=0)
        xpre_v[pl.ds(pl.multiple_of(s * 2 * PRE, 2 * PRE), 2 * PRE), :] = top.astype(BF16)
        return carry

    lax.fori_loop(0, n_seg // 2, gather_pre, 0, unroll=4)

    def prepare_pair(i, carry):
        for m in range(4):
            cp_w(i, m).wait()
        qpre_v[i] = _dot(xpre_v[...], wt_v[0, pair_rows(i), :], _NT)
        for m in range(3):
            wqkv_v[i, :, m * PW:(m + 1) * PW] = pltpu.bitcast(wt_v[m, pair_rows(i), :].T, U32)
        wo_v[i] = pltpu.bitcast(wt_v[3, pair_rows(i), :], U32)
        return carry

    lax.fori_loop(0, n_pair, prepare_pair, 0)

    b_scale = float(b_dh) ** -0.5
    h_v[seg:L, :] = mem_v[...].astype(F32)

    def b_step(s, carry):
        r0 = pl.multiple_of(s * seg, seg)
        h_v[0:seg, :] = bx_v[pl.ds(r0, seg), :].astype(F32)

        row = lax.broadcasted_iota(jnp.int32, (L, 2 * L), 0)
        col = lax.broadcasted_iota(jnp.int32, (L, 2 * L), 1)
        first = col < L
        key = jnp.where(first, col, col - L)
        mask = (row >= seg) | (key >= seg) | (key <= row)
        lo = lax.broadcasted_iota(jnp.int32, (L, LANES), 1) < b_dh - LANES

        def block_diag(t):
            z = jnp.zeros((L, LANES), F32)
            mid = t[:, LANES:2 * LANES]
            top = jnp.concatenate([t[:, 0:LANES], jnp.where(lo, mid, 0.0), z], axis=1)
            bot = jnp.concatenate([z, jnp.where(lo, 0.0, mid), t[:, 2 * LANES:]], axis=1)
            return jnp.concatenate([top, bot], axis=0).astype(BF16)

        q, kk, vv, p, o = {}, {}, {}, {}, {}
        acc = [None]

        def project(i):
            h = h_v[...]
            w = pltpu.bitcast(wqkv_v[i], BF16)
            kk[i] = block_diag(_dot(h, w[:, PW:2 * PW]))
            q[i] = jnp.concatenate([
                qpre_v[i, pl.ds(pl.multiple_of(s * PRE, PRE), PRE), :],
                _dot(h[PRE:], w[:, 0:PW])], axis=0)
            vv[i] = block_diag(_dot(h, w[:, 2 * PW:3 * PW]))

        def scores(i):
            sc = _dot(q.pop(i), kk.pop(i), _NT) * b_scale
            sc = jnp.where(mask, sc, MASK_VALUE)
            m0 = jnp.max(jnp.where(first, sc, -jnp.inf), axis=1, keepdims=True)
            m1 = jnp.max(jnp.where(first, -jnp.inf, sc), axis=1, keepdims=True)
            e = jnp.exp(sc - jnp.where(first, m0, m1))
            s0 = jnp.sum(jnp.where(first, e, 0.0), axis=1, keepdims=True)
            s1 = jnp.sum(jnp.where(first, 0.0, e), axis=1, keepdims=True)
            p[i] = e / jnp.where(first, s0, s1)

        def values(i):
            o[i] = _dot(p.pop(i), vv.pop(i))

        def out_proj(i):
            r = _dot(o.pop(i), pltpu.bitcast(wo_v[i], BF16))
            acc[0] = r if acc[0] is None else acc[0] + r

        done = 0
        i = 0
        while done < n_pair:
            if i < n_pair:
                project(i)
            if 0 <= i - D_QK < n_pair:
                scores(i - D_QK)
            if 0 <= i - D_PV < n_pair:
                values(i - D_PV)
            if i < n_pair:
                n = 1 if i >= D_WO else 0
            else:
                left = n_pair + D_PV - i
                ready = min(n_pair, i - D_PV) - done
                n = min(-(-(n_pair - 1 - done) // left), ready) if left > 0 else n_pair - done
            for _ in range(n):
                out_proj(done)
                done += 1
            i += 1

        res = acc[0].astype(BF16)
        bout_v[pl.ds(r0, seg), :] = res[0:seg]
        h_v[seg:L, :] = res[seg:L].astype(F32)
        return carry

    blk = n_seg // n_chunk

    def b_block(j, carry):
        lax.fori_loop(j * blk, (j + 1) * blk, b_step, 0)
        rows = chunk_rows(j)
        pltpu.make_async_copy(
            bout_v.at[rows], out_hbm.at[rows, pl.ds(D, D)], sem_out.at[1]).start()
        return carry

    lax.fori_loop(0, n_chunk, b_block, 0)

    cp_aout.wait()
    pltpu.make_async_copy(bout_v, out_hbm.at[:, pl.ds(D, D)], sem_out.at[1]).wait()


@functools.partial(jax.jit, static_argnames=("B_seg_len",))
def pallas_concat_heads__sliding_local_dilated__memory_aug_recurrent_mem_tr__prompt_kernel(
    A_x: jax.Array,
    A_wqkv: jax.Array,
    A_wo: jax.Array,
    B_x: jax.Array,
    B_mem0: jax.Array,
    B_Wq: jax.Array,
    B_Wk: jax.Array,
    B_Wv: jax.Array,
    B_Wo: jax.Array,
    B_seg_len: int,
):
    B, S, D = A_x.shape
    M = B_mem0.shape[1]
    _, H, Dh = B_Wq.shape
    seg = int(B_seg_len)
    assert B == 1 and B_x.shape == (B, S, D) and S % A_CHUNK == 0 and A_CHUNK % seg == 0
    assert D % LANES == 0 and D % A_HEADS == 0 and 4 * A_HEADS == LANES
    assert 2 * Dh == 3 * LANES and 2 * (seg + M) <= LANES and seg % 16 == 0 and M % 8 == 0
    n_t = D // LANES
    n_chunk = S // A_CHUNK
    assert H % 2 == 0 and (S // seg) % 2 == 0

    def head_major(w):
        return jnp.transpose(w, (1, 2, 0)).reshape(H * Dh, D)

    any_spec = pl.BlockSpec(memory_space=pl.ANY)
    out = pl.pallas_call(
        functools.partial(_kernel, seg=seg, b_heads=H, b_dh=Dh),
        in_specs=[any_spec] * 9,
        out_specs=any_spec,
        out_shape=jax.ShapeDtypeStruct((S, 2 * D), BF16),
        scratch_shapes=[
            pltpu.VMEM((S, D), BF16),
            pltpu.VMEM((3, D, D), BF16),
            pltpu.VMEM((D, D), BF16),
            pltpu.VMEM((3, D // 2, D), U32),
            pltpu.VMEM((D // 2, D), U32),
            pltpu.VMEM((n_t, D, LANES), F32),
            pltpu.VMEM((n_t, A_HALO + S, LANES), F32),
            pltpu.VMEM((n_t, A_HALO + S, LANES), F32),
            pltpu.VMEM((S, D), BF16),
            pltpu.VMEM((S, D), BF16),
            pltpu.VMEM((M, D), BF16),
            pltpu.VMEM((4, H * Dh, D), BF16),
            pltpu.VMEM((H // 2, D // 2, 6 * Dh), U32),
            pltpu.VMEM((H // 2, Dh, D), U32),
            pltpu.VMEM((S // seg * PRE, D), BF16),
            pltpu.VMEM((H // 2, S // seg * PRE, 2 * Dh), F32),
            pltpu.VMEM((seg + M, D), F32),
            pltpu.VMEM((S, D), BF16),
            pltpu.SemaphoreType.DMA((6 + n_chunk + 2 * H,)),
            pltpu.SemaphoreType.DMA((2,)),
        ],
        compiler_params=pltpu.CompilerParams(vmem_limit_bytes=112 * 1024 * 1024, flags=FLAGS),
        name="mbkern",
    )(
        A_x.reshape(S, D),
        A_wqkv,
        A_wo,
        B_x.reshape(S, D),
        B_mem0.reshape(M, D),
        head_major(B_Wq),
        head_major(B_Wk),
        head_major(B_Wv),
        B_Wo.reshape(H * Dh, D),
    )
    return out.reshape(B, S, 2 * D)
```

```python
import functools

import jax
import jax.numpy as jnp
from jax import lax
import jax.experimental.pallas as pl
import jax.experimental.pallas.tpu as pltpu

BF16 = jnp.bfloat16
F32 = jnp.float32
U32 = jnp.uint32
LANES = 128

_NN = (((1,), (0,)), ((), ()))
_NT = (((1,), (1,)), ((), ()))

A_HEADS = 32
A_WIN = 8
A_DIL = 2
A_HALO = 16
A_CHUNK = 256
A_ROWS = 64
A_D_OUT = 2
A_SUB = 16
MASK_VALUE = -1000000000.0

D_QK, D_PV, D_WO = 1, 3, 6
PRE = 8
B_UNROLL = 2
MEM_FIRST = True
P_UNROLL = 2
FLAGS = None


def _dot(a, b, dims=_NN):
    return lax.dot_general(a, b, dims, preferred_element_type=F32)


def _kernel(
    ax_hbm, awqkv_hbm, awo_hbm, bx_hbm, mem_hbm, wq_hbm, wk_hbm, wv_hbm, wo_hbm,
    out_hbm,
    ax_v, awqkv_v, awo_v, awqkv_p, awo_p, atmp_v, ak_v, av_v, aout_v,
    bx_v, mem_v, wt_v, wqkv_v, wo_v, xpre_v, qpre_v, h_v, bout_v,
    sem_in, sem_out,
    *, seg, b_heads, b_dh,
):
    S, D = ax_hbm.shape
    n_t = D // LANES
    a_dh = D // A_HEADS
    n_chunk = S // A_CHUNK
    M = mem_hbm.shape[0]
    L = seg + M
    n_seg = S // seg
    n_pair = b_heads // 2
    PW = 2 * b_dh
    w_hbm = (wq_hbm, wk_hbm, wv_hbm, wo_hbm)

    def qkv_cols(j):
        return pl.ds(pl.multiple_of(((j + 1) % 3) * D, LANES), D)

    def cp_awqkv(j):
        return pltpu.make_async_copy(awqkv_hbm.at[:, qkv_cols(j)], awqkv_v.at[j], sem_in.at[j])

    cp_awo = pltpu.make_async_copy(awo_hbm, awo_v, sem_in.at[3])
    cp_mem = pltpu.make_async_copy(mem_hbm, mem_v, sem_in.at[4])

    def chunk_rows(c):
        return pl.ds(pl.multiple_of(c * A_CHUNK, A_CHUNK), A_CHUNK)

    def cp_ax(c):
        return pltpu.make_async_copy(
            ax_hbm.at[chunk_rows(c)], ax_v.at[chunk_rows(c)], sem_in.at[6 + c])

    cp_bx = pltpu.make_async_copy(bx_hbm, bx_v, sem_in.at[5])

    def pair_rows(i):
        return pl.ds(pl.multiple_of(i * PW, PW), PW)

    def cp_w(i, m):
        return pltpu.make_async_copy(
            w_hbm[m].at[pair_rows(i)], wt_v.at[m, pair_rows(i)],
            sem_in.at[6 + n_chunk + m * n_pair + i])

    for j in range(3):
        cp_awqkv(j).start()
    cp_ax(0).start()
    cp_awo.start()
    for c in range(1, n_chunk):
        cp_ax(c).start()
    cp_mem.start()
    cp_bx.start()

    def start_w(i, carry):
        for m in range(4):
            cp_w(i, m).start()
        return carry

    lax.fori_loop(0, n_pair, start_w, 0)

    def regroup_rows(w):
        for t in range(n_t):
            atmp_v[t] = w[:, t * LANES:(t + 1) * LANES]
        return jnp.concatenate([
            jnp.concatenate(
                [atmp_v[t, pl.ds(d, A_HEADS, stride=a_dh), :] for t in range(n_t)], axis=1
            ).astype(BF16)
            for d in range(a_dh)
        ], axis=0)

    def regroup_qkv(j, carry):
        cp_awqkv(j).wait()
        awqkv_p[j] = pltpu.bitcast(regroup_rows(awqkv_v[j].astype(F32).T).T, U32)
        return carry

    lax.fori_loop(0, 3, regroup_qkv, 0)
    cp_awo.wait()
    awo_p[...] = pltpu.bitcast(regroup_rows(awo_v[...].astype(F32)), U32)

    cp_ax(0).wait()
    v0 = _dot(ax_v[0:16, :], pltpu.bitcast(awqkv_p[1], BF16))
    for t in range(n_t):
        ak_v[t, 0:A_HALO, :] = jnp.zeros((A_HALO, LANES), F32)
        av_v[t, 0:A_HALO, :] = jnp.broadcast_to(
            v0[0:1, t * LANES:(t + 1) * LANES], (A_HALO, LANES))

    a_scale = float(a_dh) ** -0.5

    def a_chunk(c, carry):
        r0 = pl.multiple_of(c * A_CHUNK, A_CHUNK)

        @pl.when(c > 0)
        def _():
            cp_ax(c).wait()

        qs, os = {}, {}

        def project(i):
            x = ax_v[pl.ds(r0 + i * A_ROWS, A_ROWS), :]
            rows = pl.ds(r0 + (A_HALO + i * A_ROWS), A_ROWS)
            for j, dst in enumerate((ak_v, av_v)):
                y = _dot(x, pltpu.bitcast(awqkv_p[j], BF16))
                for t in range(n_t):
                    dst[t, rows, :] = y[:, t * LANES:(t + 1) * LANES]
            qs[i] = _dot(x, pltpu.bitcast(awqkv_p[2], BF16))

        def attend(i):
            q = qs.pop(i)
            blocks = []
            for b in range(A_ROWS // A_SUB):
                rq = b * A_SUB
                rb = i * A_ROWS + rq
                logits = []
                for w in range(A_WIN):
                    rows = pl.ds(r0 + (A_HALO + rb - w * A_DIL), A_SUB)
                    acc = None
                    for t in range(n_t):
                        term = q[rq:rq + A_SUB, t * LANES:(t + 1) * LANES] * ak_v[t, rows, :]
                        acc = term if acc is None else acc + term
                    acc = acc + pltpu.roll(acc, 2 * A_HEADS, axis=1)
                    acc = acc + pltpu.roll(acc, A_HEADS, axis=1)
                    lg = acc * a_scale
                    if rb < w * A_DIL:
                        pos = r0 + rb + lax.broadcasted_iota(jnp.int32, (A_SUB, LANES), 0)
                        lg = jnp.where(pos >= w * A_DIL, lg, MASK_VALUE)
                    logits.append(lg)
                mx = functools.reduce(jnp.maximum, logits)
                es = [jnp.exp(lg - mx) for lg in logits]
                inv = 1.0 / functools.reduce(jnp.add, es)
                o_t = []
                for t in range(n_t):
                    acc = None
                    for w in range(A_WIN):
                        rows = pl.ds(r0 + (A_HALO + rb - w * A_DIL), A_SUB)
                        term = es[w] * av_v[t, rows, :]
                        acc = term if acc is None else acc + term
                    o_t.append((acc * inv).astype(BF16))
                blocks.append(jnp.concatenate(o_t, axis=1))
            os[i] = jnp.concatenate(blocks, axis=0)

        def out_proj(i):
            y = _dot(os.pop(i), pltpu.bitcast(awo_p[...], BF16))
            aout_v[pl.ds(r0 + i * A_ROWS, A_ROWS), :] = y.astype(BF16)

        n_sub = A_CHUNK // A_ROWS
        for i in range(n_sub + A_D_OUT):
            if i < n_sub:
                project(i)
            if 0 <= i - 1 < n_sub:
                attend(i - 1)
            if 0 <= i - A_D_OUT < n_sub:
                out_proj(i - A_D_OUT)
        return carry

    lax.fori_loop(0, n_chunk, a_chunk, 0)

    cp_aout = pltpu.make_async_copy(aout_v, out_hbm.at[:, pl.ds(0, D)], sem_out.at[0])
    cp_aout.start()

    cp_mem.wait()
    cp_bx.wait()

    def gather_pre(s, carry):
        top = jnp.concatenate([
            bx_v[pl.ds(pl.multiple_of((2 * s + u) * seg, seg), 16), :].astype(F32)[0:PRE]
            for u in range(2)], axis=0)
        xpre_v[pl.ds(pl.multiple_of(s * 2 * PRE, 2 * PRE), 2 * PRE), :] = top.astype(BF16)
        return carry

    lax.fori_loop(0, n_seg // 2, gather_pre, 0, unroll=4)

    def prepare_pairs(g, carry):
        pairs = [g * P_UNROLL + u for u in range(P_UNROLL)]
        for i in pairs:
            for m in range(4):
                cp_w(i, m).wait()
        for i in pairs:
            qpre_v[i] = _dot(xpre_v[...], wt_v[0, pair_rows(i), :], _NT)
            for m in range(3):
                wqkv_v[i, :, m * PW:(m + 1) * PW] = pltpu.bitcast(
                    wt_v[m, pair_rows(i), :].T, U32)
            wo_v[i] = pltpu.bitcast(wt_v[3, pair_rows(i), :], U32)
        return carry

    lax.fori_loop(0, n_pair // P_UNROLL, prepare_pairs, 0)

    b_scale = float(b_dh) ** -0.5
    h_v[0, seg:L, :] = mem_v[...].astype(F32)

    def b_segment(s, slot):
        r0 = pl.multiple_of(s * seg, seg)
        h_v[slot, 0:seg, :] = bx_v[pl.ds(r0, seg), :].astype(F32)

        row = lax.broadcasted_iota(jnp.int32, (L, 2 * L), 0)
        col = lax.broadcasted_iota(jnp.int32, (L, 2 * L), 1)
        first = col < L
        key = jnp.where(first, col, col - L)
        mask = (row >= seg) | (key >= seg) | (key <= row)
        lo = lax.broadcasted_iota(jnp.int32, (L, LANES), 1) < b_dh - LANES

        def block_diag(t):
            z = jnp.zeros((L, LANES), F32)
            mid = t[:, LANES:2 * LANES]
            top = jnp.concatenate([t[:, 0:LANES], jnp.where(lo, mid, 0.0), z], axis=1)
            bot = jnp.concatenate([z, jnp.where(lo, 0.0, mid), t[:, 2 * LANES:]], axis=1)
            return jnp.concatenate([top, bot], axis=0).astype(BF16)

        q, kk, vv, p, o = {}, {}, {}, {}, {}
        acc = [None]

        def project(i):
            h = h_v[slot]
            w = pltpu.bitcast(wqkv_v[i], BF16)
            kk[i] = block_diag(_dot(h, w[:, PW:2 * PW]))
            q[i] = jnp.concatenate([
                qpre_v[i, pl.ds(pl.multiple_of(s * PRE, PRE), PRE), :],
                _dot(h[PRE:], w[:, 0:PW])], axis=0)
            vv[i] = block_diag(_dot(h, w[:, 2 * PW:3 * PW]))

        def scores(i):
            sc = _dot(q.pop(i), kk.pop(i), _NT) * b_scale
            sc = jnp.where(mask, sc, MASK_VALUE)
            m0 = jnp.max(jnp.where(first, sc, -jnp.inf), axis=1, keepdims=True)
            m1 = jnp.max(jnp.where(first, -jnp.inf, sc), axis=1, keepdims=True)
            e = jnp.exp(sc - jnp.where(first, m0, m1))
            s0 = jnp.sum(jnp.where(first, e, 0.0), axis=1, keepdims=True)
            s1 = jnp.sum(jnp.where(first, 0.0, e), axis=1, keepdims=True)
            p[i] = e / jnp.where(first, s0, s1)

        def values(i):
            o[i] = _dot(p.pop(i), vv.pop(i))

        def out_proj(i):
            oi = o.pop(i)
            if MEM_FIRST:
                oi = jnp.concatenate([oi[seg:], oi[:seg]], axis=0)
            r = _dot(oi, pltpu.bitcast(wo_v[i], BF16))
            acc[0] = r if acc[0] is None else acc[0] + r

        done = 0
        i = 0
        while done < n_pair:
            if i < n_pair:
                project(i)
            if 0 <= i - D_QK < n_pair:
                scores(i - D_QK)
            if 0 <= i - D_PV < n_pair:
                values(i - D_PV)
            if i < n_pair:
                n = 1 if i >= D_WO else 0
            else:
                left = n_pair + D_PV - i
                ready = min(n_pair, i - D_PV) - done
                n = min(-(-(n_pair - 1 - done) // left), ready) if left > 0 else n_pair - done
            for _ in range(n):
                out_proj(done)
                done += 1
            i += 1

        new_mem, res = (acc[0][:M], acc[0][M:]) if MEM_FIRST else (acc[0][seg:], acc[0][:seg])
        h_v[(slot + 1) % B_UNROLL, seg:L, :] = new_mem
        bout_v[pl.ds(r0, seg), :] = res.astype(BF16)

    def b_step(g, carry):
        for u in range(B_UNROLL):
            b_segment(g * B_UNROLL + u, u)
        return carry

    blk = n_seg // n_chunk // B_UNROLL

    def b_block(j, carry):
        lax.fori_loop(j * blk, (j + 1) * blk, b_step, 0)
        rows = chunk_rows(j)
        pltpu.make_async_copy(
            bout_v.at[rows], out_hbm.at[rows, pl.ds(D, D)], sem_out.at[1]).start()
        return carry

    lax.fori_loop(0, n_chunk, b_block, 0)

    cp_aout.wait()
    pltpu.make_async_copy(bout_v, out_hbm.at[:, pl.ds(D, D)], sem_out.at[1]).wait()


@functools.partial(jax.jit, static_argnames=("B_seg_len",))
def pallas_concat_heads__sliding_local_dilated__memory_aug_recurrent_mem_tr__prompt_kernel(
    A_x: jax.Array,
    A_wqkv: jax.Array,
    A_wo: jax.Array,
    B_x: jax.Array,
    B_mem0: jax.Array,
    B_Wq: jax.Array,
    B_Wk: jax.Array,
    B_Wv: jax.Array,
    B_Wo: jax.Array,
    B_seg_len: int,
):
    B, S, D = A_x.shape
    M = B_mem0.shape[1]
    _, H, Dh = B_Wq.shape
    seg = int(B_seg_len)
    assert B == 1 and B_x.shape == (B, S, D) and S % A_CHUNK == 0 and A_CHUNK % seg == 0
    assert D % LANES == 0 and D % A_HEADS == 0 and 4 * A_HEADS == LANES
    assert 2 * Dh == 3 * LANES and 2 * (seg + M) <= LANES and seg % 16 == 0 and M % 8 == 0
    n_t = D // LANES
    n_chunk = S // A_CHUNK
    assert H % 2 == 0 and (S // seg) % 2 == 0

    def head_major(w):
        return jnp.transpose(w, (1, 2, 0)).reshape(H * Dh, D)

    any_spec = pl.BlockSpec(memory_space=pl.ANY)
    out = pl.pallas_call(
        functools.partial(_kernel, seg=seg, b_heads=H, b_dh=Dh),
        in_specs=[any_spec] * 9,
        out_specs=any_spec,
        out_shape=jax.ShapeDtypeStruct((S, 2 * D), BF16),
        scratch_shapes=[
            pltpu.VMEM((S, D), BF16),
            pltpu.VMEM((3, D, D), BF16),
            pltpu.VMEM((D, D), BF16),
            pltpu.VMEM((3, D // 2, D), U32),
            pltpu.VMEM((D // 2, D), U32),
            pltpu.VMEM((n_t, D, LANES), F32),
            pltpu.VMEM((n_t, A_HALO + S, LANES), F32),
            pltpu.VMEM((n_t, A_HALO + S, LANES), F32),
            pltpu.VMEM((S, D), BF16),
            pltpu.VMEM((S, D), BF16),
            pltpu.VMEM((M, D), BF16),
            pltpu.VMEM((4, H * Dh, D), BF16),
            pltpu.VMEM((H // 2, D // 2, 6 * Dh), U32),
            pltpu.VMEM((H // 2, Dh, D), U32),
            pltpu.VMEM((S // seg * PRE, D), BF16),
            pltpu.VMEM((H // 2, S // seg * PRE, 2 * Dh), F32),
            pltpu.VMEM((B_UNROLL, seg + M, D), F32),
            pltpu.VMEM((S, D), BF16),
            pltpu.SemaphoreType.DMA((6 + n_chunk + 2 * H,)),
            pltpu.SemaphoreType.DMA((2,)),
        ],
        compiler_params=pltpu.CompilerParams(vmem_limit_bytes=112 * 1024 * 1024, flags=FLAGS),
        name="mbkern",
    )(
        A_x.reshape(S, D),
        A_wqkv,
        A_wo,
        B_x.reshape(S, D),
        B_mem0.reshape(M, D),
        head_major(B_Wq),
        head_major(B_Wk),
        head_major(B_Wv),
        B_Wo.reshape(H * Dh, D),
    )
    return out.reshape(B, S, 2 * D)
```

```python
import functools

import jax
import jax.numpy as jnp
from jax import lax
import jax.experimental.pallas as pl
import jax.experimental.pallas.tpu as pltpu

BF16 = jnp.bfloat16
F32 = jnp.float32
U32 = jnp.uint32
LANES = 128

_NN = (((1,), (0,)), ((), ()))
_NT = (((1,), (1,)), ((), ()))

A_HEADS = 32
A_WIN = 8
A_DIL = 2
A_HALO = 16
A_CHUNK = 512
A_ROWS = 64
A_D_OUT = 3
A_SUB = 16
MASK_VALUE = -1000000000.0

D_QK, D_PV, D_WO = 1, 3, 6
PRE = 8
B_UNROLL = 4
MEM_FIRST = True
P_UNROLL = 4
FLAGS = None


def _dot(a, b, dims=_NN):
    return lax.dot_general(a, b, dims, preferred_element_type=F32)


def _kernel(
    ax_hbm, awqkv_hbm, awo_hbm, bx_hbm, mem_hbm, wq_hbm, wk_hbm, wv_hbm, wo_hbm,
    out_hbm,
    ax_v, awqkv_v, awo_v, awqkv_p, awo_p, atmp_v, ak_v, av_v, aout_v,
    bx_v, mem_v, wt_v, wqkv_v, wo_v, xpre_v, qpre_v, h_v, bout_v,
    sem_in, sem_out,
    *, seg, b_heads, b_dh,
):
    S, D = ax_hbm.shape
    n_t = D // LANES
    a_dh = D // A_HEADS
    n_chunk = S // A_CHUNK
    M = mem_hbm.shape[0]
    L = seg + M
    n_seg = S // seg
    n_pair = b_heads // 2
    PW = 2 * b_dh
    w_hbm = (wq_hbm, wk_hbm, wv_hbm, wo_hbm)

    def qkv_cols(j):
        return pl.ds(pl.multiple_of(((j + 1) % 3) * D, LANES), D)

    def cp_awqkv(j):
        return pltpu.make_async_copy(awqkv_hbm.at[:, qkv_cols(j)], awqkv_v.at[j], sem_in.at[j])

    cp_awo = pltpu.make_async_copy(awo_hbm, awo_v, sem_in.at[3])
    cp_mem = pltpu.make_async_copy(mem_hbm, mem_v, sem_in.at[4])

    def chunk_rows(c):
        return pl.ds(pl.multiple_of(c * A_CHUNK, A_CHUNK), A_CHUNK)

    def cp_ax(c):
        return pltpu.make_async_copy(
            ax_hbm.at[chunk_rows(c)], ax_v.at[chunk_rows(c)], sem_in.at[6 + c])

    cp_bx = pltpu.make_async_copy(bx_hbm, bx_v, sem_in.at[5])

    def pair_rows(i):
        return pl.ds(pl.multiple_of(i * PW, PW), PW)

    n_group = n_pair // P_UNROLL

    def cp_w(g, m):
        rows = pl.ds(pl.multiple_of(g * (P_UNROLL * PW), P_UNROLL * PW), P_UNROLL * PW)
        return pltpu.make_async_copy(
            w_hbm[m].at[rows], wt_v.at[m, rows], sem_in.at[6 + n_chunk + g])

    for j in range(3):
        cp_awqkv(j).start()
    cp_awo.start()
    for c in range(n_chunk):
        cp_ax(c).start()
    cp_mem.start()
    cp_bx.start()
    for g in range(n_group):
        for m in range(4):
            cp_w(g, m).start()

    def regroup_rows(w):
        for t in range(n_t):
            atmp_v[t] = w[:, t * LANES:(t + 1) * LANES]
        return jnp.concatenate([
            jnp.concatenate(
                [atmp_v[t, pl.ds(d, A_HEADS, stride=a_dh), :] for t in range(n_t)], axis=1
            ).astype(BF16)
            for d in range(a_dh)
        ], axis=0)

    def regroup_qkv(j, carry):
        cp_awqkv(j).wait()
        awqkv_p[j] = pltpu.bitcast(regroup_rows(awqkv_v[j].astype(F32).T).T, U32)
        return carry

    lax.fori_loop(0, 3, regroup_qkv, 0)
    cp_awo.wait()
    awo_p[...] = pltpu.bitcast(regroup_rows(awo_v[...].astype(F32)), U32)

    cp_ax(0).wait()
    v0 = _dot(ax_v[0:16, :], pltpu.bitcast(awqkv_p[1], BF16))
    for t in range(n_t):
        ak_v[t, 0:A_HALO, :] = jnp.zeros((A_HALO, LANES), F32)
        av_v[t, 0:A_HALO, :] = jnp.broadcast_to(
            v0[0:1, t * LANES:(t + 1) * LANES], (A_HALO, LANES))

    a_scale = float(a_dh) ** -0.5

    def a_chunk(c, carry):
        r0 = pl.multiple_of(c * A_CHUNK, A_CHUNK)

        @pl.when(c > 0)
        def _():
            cp_ax(c).wait()

        qs, os = {}, {}

        def project(i):
            x = ax_v[pl.ds(r0 + i * A_ROWS, A_ROWS), :]
            rows = pl.ds(r0 + (A_HALO + i * A_ROWS), A_ROWS)
            for j, dst in enumerate((ak_v, av_v)):
                y = _dot(x, pltpu.bitcast(awqkv_p[j], BF16))
                for t in range(n_t):
                    dst[t, rows, :] = y[:, t * LANES:(t + 1) * LANES]
            qs[i] = _dot(x, pltpu.bitcast(awqkv_p[2], BF16))

        def attend(i):
            q = qs.pop(i)
            blocks = []
            for b in range(A_ROWS // A_SUB):
                rq = b * A_SUB
                rb = i * A_ROWS + rq
                logits = []
                for w in range(A_WIN):
                    rows = pl.ds(r0 + (A_HALO + rb - w * A_DIL), A_SUB)
                    acc = None
                    for t in range(n_t):
                        term = q[rq:rq + A_SUB, t * LANES:(t + 1) * LANES] * ak_v[t, rows, :]
                        acc = term if acc is None else acc + term
                    acc = acc + pltpu.roll(acc, 2 * A_HEADS, axis=1)
                    acc = acc + pltpu.roll(acc, A_HEADS, axis=1)
                    lg = acc * a_scale
                    if rb < w * A_DIL:
                        pos = r0 + rb + lax.broadcasted_iota(jnp.int32, (A_SUB, LANES), 0)
                        lg = jnp.where(pos >= w * A_DIL, lg, MASK_VALUE)
                    logits.append(lg)
                mx = functools.reduce(jnp.maximum, logits)
                es = [jnp.exp(lg - mx) for lg in logits]
                inv = 1.0 / functools.reduce(jnp.add, es)
                o_t = []
                for t in range(n_t):
                    acc = None
                    for w in range(A_WIN):
                        rows = pl.ds(r0 + (A_HALO + rb - w * A_DIL), A_SUB)
                        term = es[w] * av_v[t, rows, :]
                        acc = term if acc is None else acc + term
                    o_t.append((acc * inv).astype(BF16))
                blocks.append(jnp.concatenate(o_t, axis=1))
            os[i] = jnp.concatenate(blocks, axis=0)

        def out_proj(i):
            y = _dot(os.pop(i), pltpu.bitcast(awo_p[...], BF16))
            aout_v[pl.ds(r0 + i * A_ROWS, A_ROWS), :] = y.astype(BF16)

        n_sub = A_CHUNK // A_ROWS
        for i in range(n_sub + A_D_OUT):
            if i < n_sub:
                project(i)
            if 0 <= i - 1 < n_sub:
                attend(i - 1)
            if 0 <= i - A_D_OUT < n_sub:
                out_proj(i - A_D_OUT)
        return carry

    lax.fori_loop(0, n_chunk, a_chunk, 0)

    cp_aout = pltpu.make_async_copy(aout_v, out_hbm.at[:, pl.ds(0, D)], sem_out.at[0])
    cp_aout.start()

    cp_mem.wait()
    cp_bx.wait()

    def gather_pre(s, carry):
        top = jnp.concatenate([
            bx_v[pl.ds(pl.multiple_of((2 * s + u) * seg, seg), 16), :].astype(F32)[0:PRE]
            for u in range(2)], axis=0)
        xpre_v[pl.ds(pl.multiple_of(s * 2 * PRE, 2 * PRE), 2 * PRE), :] = top.astype(BF16)
        return carry

    lax.fori_loop(0, n_seg // 2, gather_pre, 0, unroll=4)

    def prepare_pairs(g, carry):
        for m in range(4):
            cp_w(g, m).wait()
        for i in [g * P_UNROLL + u for u in range(P_UNROLL)]:
            qpre_v[i] = _dot(xpre_v[...], wt_v[0, pair_rows(i), :], _NT)
            for m in range(3):
                wqkv_v[i, :, m * PW:(m + 1) * PW] = pltpu.bitcast(
                    wt_v[m, pair_rows(i), :].T, U32)
            wo_v[i] = pltpu.bitcast(wt_v[3, pair_rows(i), :], U32)
        return carry

    lax.fori_loop(0, n_group, prepare_pairs, 0)

    b_scale = float(b_dh) ** -0.5
    h_v[0, seg:L, :] = mem_v[...].astype(F32)

    def b_segment(s, slot):
        r0 = pl.multiple_of(s * seg, seg)
        h_v[slot, 0:seg, :] = bx_v[pl.ds(r0, seg), :].astype(F32)

        row = lax.broadcasted_iota(jnp.int32, (L, 2 * L), 0)
        col = lax.broadcasted_iota(jnp.int32, (L, 2 * L), 1)
        first = col < L
        key = jnp.where(first, col, col - L)
        mask = (row >= seg) | (key >= seg) | (key <= row)
        lo = lax.broadcasted_iota(jnp.int32, (L, LANES), 1) < b_dh - LANES

        def block_diag(t):
            z = jnp.zeros((L, LANES), F32)
            mid = t[:, LANES:2 * LANES]
            top = jnp.concatenate([t[:, 0:LANES], jnp.where(lo, mid, 0.0), z], axis=1)
            bot = jnp.concatenate([z, jnp.where(lo, 0.0, mid), t[:, 2 * LANES:]], axis=1)
            return jnp.concatenate([top, bot], axis=0).astype(BF16)

        q, kk, vv, p, o = {}, {}, {}, {}, {}
        acc = [None]

        def project(i):
            h = h_v[slot]
            w = pltpu.bitcast(wqkv_v[i], BF16)
            if i == 0 and slot > 0:
                k = functools.reduce(jnp.add, [
                    _dot(h[:, t * LANES:(t + 1) * LANES], w[t * LANES:(t + 1) * LANES, PW:2 * PW])
                    for t in range(n_t)])
            else:
                k = _dot(h, w[:, PW:2 * PW])
            kk[i] = block_diag(k)
            q[i] = jnp.concatenate([
                qpre_v[i, pl.ds(pl.multiple_of(s * PRE, PRE), PRE), :],
                _dot(h[PRE:], w[:, 0:PW])], axis=0)
            vv[i] = block_diag(_dot(h, w[:, 2 * PW:3 * PW]))

        def scores(i):
            sc = _dot(q.pop(i), kk.pop(i), _NT) * b_scale
            sc = jnp.where(mask, sc, MASK_VALUE)
            m0 = jnp.max(jnp.where(first, sc, -jnp.inf), axis=1, keepdims=True)
            m1 = jnp.max(jnp.where(first, -jnp.inf, sc), axis=1, keepdims=True)
            e = jnp.exp(sc - jnp.where(first, m0, m1))
            s0 = jnp.sum(jnp.where(first, e, 0.0), axis=1, keepdims=True)
            s1 = jnp.sum(jnp.where(first, 0.0, e), axis=1, keepdims=True)
            p[i] = e / jnp.where(first, s0, s1)

        def values(i):
            o[i] = _dot(p.pop(i), vv.pop(i))

        def out_proj(i):
            oi = o.pop(i)
            if MEM_FIRST:
                oi = jnp.concatenate([oi[seg:], oi[:seg]], axis=0)
            r = _dot(oi, pltpu.bitcast(wo_v[i], BF16))
            acc[0] = r if acc[0] is None else acc[0] + r

        done = 0
        i = 0
        while done < n_pair:
            if i < n_pair:
                project(i)
            if 0 <= i - D_QK < n_pair:
                scores(i - D_QK)
            if 0 <= i - D_PV < n_pair:
                values(i - D_PV)
            if i < n_pair:
                n = 1 if i >= D_WO else 0
            else:
                left = n_pair + D_PV - i
                ready = min(n_pair, i - D_PV) - done
                n = min(-(-(n_pair - 1 - done) // left), ready) if left > 0 else n_pair - done
            for _ in range(n):
                out_proj(done)
                done += 1
            i += 1

        new_mem, res = (acc[0][:M], acc[0][M:]) if MEM_FIRST else (acc[0][seg:], acc[0][:seg])
        h_v[(slot + 1) % B_UNROLL, seg:L, :] = new_mem
        rows = pl.ds(r0, seg)
        bout_v[rows, :] = res.astype(BF16)
        pltpu.make_async_copy(
            bout_v.at[rows], out_hbm.at[rows, pl.ds(D, D)], sem_out.at[1]).start()

    def b_step(g, carry):
        for u in range(B_UNROLL):
            b_segment(g * B_UNROLL + u, u)
        return carry

    lax.fori_loop(0, n_seg // B_UNROLL, b_step, 0)

    cp_aout.wait()
    pltpu.make_async_copy(bout_v, out_hbm.at[:, pl.ds(D, D)], sem_out.at[1]).wait()


@functools.partial(jax.jit, static_argnames=("B_seg_len",))
def pallas_concat_heads__sliding_local_dilated__memory_aug_recurrent_mem_tr__prompt_kernel(
    A_x: jax.Array,
    A_wqkv: jax.Array,
    A_wo: jax.Array,
    B_x: jax.Array,
    B_mem0: jax.Array,
    B_Wq: jax.Array,
    B_Wk: jax.Array,
    B_Wv: jax.Array,
    B_Wo: jax.Array,
    B_seg_len: int,
):
    B, S, D = A_x.shape
    M = B_mem0.shape[1]
    _, H, Dh = B_Wq.shape
    seg = int(B_seg_len)
    assert B == 1 and B_x.shape == (B, S, D) and S % A_CHUNK == 0 and A_CHUNK % seg == 0
    assert D % LANES == 0 and D % A_HEADS == 0 and 4 * A_HEADS == LANES
    assert 2 * Dh == 3 * LANES and 2 * (seg + M) <= LANES and seg % 16 == 0 and M % 8 == 0
    n_t = D // LANES
    n_chunk = S // A_CHUNK
    assert H % 2 == 0 and (S // seg) % 2 == 0

    def head_major(w):
        return jnp.transpose(w, (1, 2, 0)).reshape(H * Dh, D)

    any_spec = pl.BlockSpec(memory_space=pl.ANY)
    out = pl.pallas_call(
        functools.partial(_kernel, seg=seg, b_heads=H, b_dh=Dh),
        in_specs=[any_spec] * 9,
        out_specs=any_spec,
        out_shape=jax.ShapeDtypeStruct((S, 2 * D), BF16),
        scratch_shapes=[
            pltpu.VMEM((S, D), BF16),
            pltpu.VMEM((3, D, D), BF16),
            pltpu.VMEM((D, D), BF16),
            pltpu.VMEM((3, D // 2, D), U32),
            pltpu.VMEM((D // 2, D), U32),
            pltpu.VMEM((n_t, D, LANES), F32),
            pltpu.VMEM((n_t, A_HALO + S, LANES), F32),
            pltpu.VMEM((n_t, A_HALO + S, LANES), F32),
            pltpu.VMEM((S, D), BF16),
            pltpu.VMEM((S, D), BF16),
            pltpu.VMEM((M, D), BF16),
            pltpu.VMEM((4, H * Dh, D), BF16),
            pltpu.VMEM((H // 2, D // 2, 6 * Dh), U32),
            pltpu.VMEM((H // 2, Dh, D), U32),
            pltpu.VMEM((S // seg * PRE, D), BF16),
            pltpu.VMEM((H // 2, S // seg * PRE, 2 * Dh), F32),
            pltpu.VMEM((B_UNROLL, seg + M, D), F32),
            pltpu.VMEM((S, D), BF16),
            pltpu.SemaphoreType.DMA((6 + n_chunk + H // 2 // P_UNROLL,)),
            pltpu.SemaphoreType.DMA((2,)),
        ],
        compiler_params=pltpu.CompilerParams(vmem_limit_bytes=112 * 1024 * 1024, flags=FLAGS),
        name="mbkern",
    )(
        A_x.reshape(S, D),
        A_wqkv,
        A_wo,
        B_x.reshape(S, D),
        B_mem0.reshape(M, D),
        head_major(B_Wq),
        head_major(B_Wk),
        head_major(B_Wv),
        B_Wo.reshape(H * Dh, D),
    )
    return out.reshape(B, S, 2 * D)
```

```python
import functools

import jax
import jax.numpy as jnp
from jax import lax
import jax.experimental.pallas as pl
import jax.experimental.pallas.tpu as pltpu

BF16 = jnp.bfloat16
F32 = jnp.float32
U32 = jnp.uint32
LANES = 128

_NN = (((1,), (0,)), ((), ()))
_NT = (((1,), (1,)), ((), ()))

A_HEADS = 32
A_WIN = 8
A_DIL = 2
A_HALO = 16
A_CHUNK = 512
A_ROWS = 64
A_D_OUT = 3
A_SUB = 16
MASK_VALUE = -1000000000.0

D_QK, D_PV, D_WO = 1, 3, 6
PRE = 8
B_UNROLL = 4
MEM_FIRST = True
P_UNROLL = 4
FLAGS = None


def _dot(a, b, dims=_NN):
    return lax.dot_general(a, b, dims, preferred_element_type=F32)


def _kernel(
    ax_hbm, awqkv_hbm, awo_hbm, bx_hbm, mem_hbm, wq_hbm, wk_hbm, wv_hbm, wo_hbm,
    out_hbm,
    ax_v, awqkv_v, awo_v, awqkv_p, awo_p, atmp_v, ak_v, av_v, aout_v,
    bx_v, mem_v, wt_v, wqkv_v, wo_v, xpre_v, qpre_v, h_v, bout_v,
    sem_in, sem_out,
    *, seg, b_heads, b_dh,
):
    S, D = ax_hbm.shape
    n_t = D // LANES
    a_dh = D // A_HEADS
    n_chunk = S // A_CHUNK
    M = mem_hbm.shape[0]
    L = seg + M
    n_seg = S // seg
    n_pair = b_heads // 2
    PW = 2 * b_dh
    w_hbm = (wq_hbm, wk_hbm, wv_hbm, wo_hbm)

    def qkv_cols(j):
        return pl.ds(pl.multiple_of(((j + 1) % 3) * D, LANES), D)

    def cp_awqkv(j):
        return pltpu.make_async_copy(awqkv_hbm.at[:, qkv_cols(j)], awqkv_v.at[j], sem_in.at[j])

    cp_awo = pltpu.make_async_copy(awo_hbm, awo_v, sem_in.at[3])
    cp_mem = pltpu.make_async_copy(mem_hbm, mem_v, sem_in.at[4])

    def chunk_rows(c):
        return pl.ds(pl.multiple_of(c * A_CHUNK, A_CHUNK), A_CHUNK)

    def cp_ax(c):
        return pltpu.make_async_copy(
            ax_hbm.at[chunk_rows(c)], ax_v.at[chunk_rows(c)], sem_in.at[6 + c])

    cp_bx = pltpu.make_async_copy(bx_hbm, bx_v, sem_in.at[5])

    def pair_rows(i):
        return pl.ds(pl.multiple_of(i * PW, PW), PW)

    n_group = n_pair // P_UNROLL

    def cp_w(g, m):
        rows = pl.ds(pl.multiple_of(g * (P_UNROLL * PW), P_UNROLL * PW), P_UNROLL * PW)
        return pltpu.make_async_copy(
            w_hbm[m].at[rows], wt_v.at[m, rows], sem_in.at[6 + n_chunk + g])

    for j in range(3):
        cp_awqkv(j).start()
    cp_awo.start()
    for c in range(n_chunk):
        cp_ax(c).start()
    cp_mem.start()
    cp_bx.start()
    for g in range(n_group):
        for m in range(4):
            cp_w(g, m).start()

    def regroup_rows(w):
        for t in range(n_t):
            atmp_v[t] = w[:, t * LANES:(t + 1) * LANES]
        return jnp.concatenate([
            jnp.concatenate(
                [atmp_v[t, pl.ds(d, A_HEADS, stride=a_dh), :] for t in range(n_t)], axis=1
            ).astype(BF16)
            for d in range(a_dh)
        ], axis=0)

    def regroup_qkv(j, carry):
        cp_awqkv(j).wait()
        awqkv_p[j] = pltpu.bitcast(regroup_rows(awqkv_v[j].astype(F32).T).T, U32)
        return carry

    lax.fori_loop(0, 3, regroup_qkv, 0)
    cp_awo.wait()
    awo_p[...] = pltpu.bitcast(regroup_rows(awo_v[...].astype(F32)), U32)

    cp_ax(0).wait()
    v0 = _dot(ax_v[0:16, :], pltpu.bitcast(awqkv_p[1], BF16))
    for t in range(n_t):
        ak_v[t, 0:A_HALO, :] = jnp.zeros((A_HALO, LANES), F32)
        av_v[t, 0:A_HALO, :] = jnp.broadcast_to(
            v0[0:1, t * LANES:(t + 1) * LANES], (A_HALO, LANES))

    a_scale = float(a_dh) ** -0.5

    def a_chunk(c, carry):
        r0 = pl.multiple_of(c * A_CHUNK, A_CHUNK)

        @pl.when(c > 0)
        def _():
            cp_ax(c).wait()

        qs, os = {}, {}

        def project(i):
            x = ax_v[pl.ds(r0 + i * A_ROWS, A_ROWS), :]
            rows = pl.ds(A_HALO + i * A_ROWS, A_ROWS)
            for j, dst in enumerate((ak_v, av_v)):
                y = _dot(x, pltpu.bitcast(awqkv_p[j], BF16))
                for t in range(n_t):
                    dst[t, rows, :] = y[:, t * LANES:(t + 1) * LANES]
            qs[i] = _dot(x, pltpu.bitcast(awqkv_p[2], BF16))

        def attend(i):
            q = qs.pop(i)
            blocks = []
            for b in range(A_ROWS // A_SUB):
                rq = b * A_SUB
                rb = i * A_ROWS + rq
                logits = []
                for w in range(A_WIN):
                    rows = pl.ds(A_HALO + rb - w * A_DIL, A_SUB)
                    acc = None
                    for t in range(n_t):
                        term = q[rq:rq + A_SUB, t * LANES:(t + 1) * LANES] * ak_v[t, rows, :]
                        acc = term if acc is None else acc + term
                    acc = acc + pltpu.roll(acc, 2 * A_HEADS, axis=1)
                    acc = acc + pltpu.roll(acc, A_HEADS, axis=1)
                    lg = acc * a_scale
                    if rb < w * A_DIL:
                        pos = r0 + rb + lax.broadcasted_iota(jnp.int32, (A_SUB, LANES), 0)
                        lg = jnp.where(pos >= w * A_DIL, lg, MASK_VALUE)
                    logits.append(lg)
                mx = functools.reduce(jnp.maximum, logits)
                es = [jnp.exp(lg - mx) for lg in logits]
                inv = 1.0 / functools.reduce(jnp.add, es)
                o_t = []
                for t in range(n_t):
                    acc = None
                    for w in range(A_WIN):
                        rows = pl.ds(A_HALO + rb - w * A_DIL, A_SUB)
                        term = es[w] * av_v[t, rows, :]
                        acc = term if acc is None else acc + term
                    o_t.append((acc * inv).astype(BF16))
                blocks.append(jnp.concatenate(o_t, axis=1))
            os[i] = jnp.concatenate(blocks, axis=0)

        def out_proj(i):
            y = _dot(os.pop(i), pltpu.bitcast(awo_p[...], BF16))
            aout_v[pl.ds(r0 + i * A_ROWS, A_ROWS), :] = y.astype(BF16)

        n_sub = A_CHUNK // A_ROWS
        for i in range(n_sub + A_D_OUT):
            if i < n_sub:
                project(i)
            if 0 <= i - 1 < n_sub:
                attend(i - 1)
            if 0 <= i - A_D_OUT < n_sub:
                out_proj(i - A_D_OUT)
        for buf in (ak_v, av_v):
            buf[:, 0:A_HALO, :] = buf[:, A_CHUNK:A_CHUNK + A_HALO, :]
        return carry

    lax.fori_loop(0, n_chunk, a_chunk, 0)

    cp_aout = pltpu.make_async_copy(aout_v, out_hbm.at[:, pl.ds(0, D)], sem_out.at[0])
    cp_aout.start()

    cp_mem.wait()
    cp_bx.wait()

    def gather_pre(s, carry):
        top = jnp.concatenate([
            bx_v[pl.ds(pl.multiple_of((2 * s + u) * seg, seg), 16), :].astype(F32)[0:PRE]
            for u in range(2)], axis=0)
        xpre_v[pl.ds(pl.multiple_of(s * 2 * PRE, 2 * PRE), 2 * PRE), :] = top.astype(BF16)
        return carry

    lax.fori_loop(0, n_seg // 2, gather_pre, 0, unroll=4)

    def prepare_pairs(g, carry):
        for m in range(4):
            cp_w(g, m).wait()
        for i in [g * P_UNROLL + u for u in range(P_UNROLL)]:
            qpre_v[i] = _dot(xpre_v[...], wt_v[0, pair_rows(i), :], _NT)
            for m in range(3):
                wqkv_v[i, :, m * PW:(m + 1) * PW] = pltpu.bitcast(
                    wt_v[m, pair_rows(i), :].T, U32)
            wo_v[i] = pltpu.bitcast(wt_v[3, pair_rows(i), :], U32)
        return carry

    lax.fori_loop(0, n_group, prepare_pairs, 0)

    b_scale = float(b_dh) ** -0.5
    h_v[0, seg:L, :] = mem_v[...].astype(F32)

    def b_segment(s, slot):
        r0 = pl.multiple_of(s * seg, seg)
        h_v[slot, 0:seg, :] = bx_v[pl.ds(r0, seg), :].astype(F32)

        row = lax.broadcasted_iota(jnp.int32, (L, 2 * L), 0)
        col = lax.broadcasted_iota(jnp.int32, (L, 2 * L), 1)
        first = col < L
        key = jnp.where(first, col, col - L)
        mask = (row >= seg) | (key >= seg) | (key <= row)
        lo = lax.broadcasted_iota(jnp.int32, (L, LANES), 1) < b_dh - LANES

        def block_diag(t):
            z = jnp.zeros((L, LANES), F32)
            mid = t[:, LANES:2 * LANES]
            top = jnp.concatenate([t[:, 0:LANES], jnp.where(lo, mid, 0.0), z], axis=1)
            bot = jnp.concatenate([z, jnp.where(lo, 0.0, mid), t[:, 2 * LANES:]], axis=1)
            return jnp.concatenate([top, bot], axis=0).astype(BF16)

        q, kk, vv, p, o = {}, {}, {}, {}, {}
        acc = [None]

        def project(i):
            h = h_v[slot]
            w = pltpu.bitcast(wqkv_v[i], BF16)
            if i == 0 and slot > 0:
                k = functools.reduce(jnp.add, [
                    _dot(h[:, t * LANES:(t + 1) * LANES], w[t * LANES:(t + 1) * LANES, PW:2 * PW])
                    for t in range(n_t)])
            else:
                k = _dot(h, w[:, PW:2 * PW])
            kk[i] = block_diag(k)
            q[i] = jnp.concatenate([
                qpre_v[i, pl.ds(pl.multiple_of(s * PRE, PRE), PRE), :],
                _dot(h[PRE:], w[:, 0:PW])], axis=0)
            vv[i] = block_diag(_dot(h, w[:, 2 * PW:3 * PW]))

        def scores(i):
            sc = _dot(q.pop(i), kk.pop(i), _NT) * b_scale
            sc = jnp.where(mask, sc, MASK_VALUE)
            m0 = jnp.max(jnp.where(first, sc, -jnp.inf), axis=1, keepdims=True)
            m1 = jnp.max(jnp.where(first, -jnp.inf, sc), axis=1, keepdims=True)
            e = jnp.exp(sc - jnp.where(first, m0, m1))
            s0 = jnp.sum(jnp.where(first, e, 0.0), axis=1, keepdims=True)
            s1 = jnp.sum(jnp.where(first, 0.0, e), axis=1, keepdims=True)
            p[i] = e / jnp.where(first, s0, s1)

        def values(i):
            o[i] = _dot(p.pop(i), vv.pop(i))

        def out_proj(i):
            oi = o.pop(i)
            if MEM_FIRST:
                oi = jnp.concatenate([oi[seg:], oi[:seg]], axis=0)
            r = _dot(oi, pltpu.bitcast(wo_v[i], BF16))
            acc[0] = r if acc[0] is None else acc[0] + r

        done = 0
        i = 0
        while done < n_pair:
            if i < n_pair:
                project(i)
            if 0 <= i - D_QK < n_pair:
                scores(i - D_QK)
            if 0 <= i - D_PV < n_pair:
                values(i - D_PV)
            if i < n_pair:
                n = 1 if i >= D_WO else 0
            else:
                left = n_pair + D_PV - i
                ready = min(n_pair, i - D_PV) - done
                n = min(-(-(n_pair - 1 - done) // left), ready) if left > 0 else n_pair - done
            for _ in range(n):
                out_proj(done)
                done += 1
            i += 1

        new_mem, res = (acc[0][:M], acc[0][M:]) if MEM_FIRST else (acc[0][seg:], acc[0][:seg])
        h_v[(slot + 1) % B_UNROLL, seg:L, :] = new_mem
        rows = pl.ds(r0, seg)
        bout_v[rows, :] = res.astype(BF16)
        pltpu.make_async_copy(
            bout_v.at[rows], out_hbm.at[rows, pl.ds(D, D)], sem_out.at[1]).start()

    def b_step(g, carry):
        for u in range(B_UNROLL):
            b_segment(g * B_UNROLL + u, u)
        return carry

    lax.fori_loop(0, n_seg // B_UNROLL, b_step, 0)

    cp_aout.wait()
    pltpu.make_async_copy(bout_v, out_hbm.at[:, pl.ds(D, D)], sem_out.at[1]).wait()


@functools.partial(jax.jit, static_argnames=("B_seg_len",))
def pallas_concat_heads__sliding_local_dilated__memory_aug_recurrent_mem_tr__prompt_kernel(
    A_x: jax.Array,
    A_wqkv: jax.Array,
    A_wo: jax.Array,
    B_x: jax.Array,
    B_mem0: jax.Array,
    B_Wq: jax.Array,
    B_Wk: jax.Array,
    B_Wv: jax.Array,
    B_Wo: jax.Array,
    B_seg_len: int,
):
    B, S, D = A_x.shape
    M = B_mem0.shape[1]
    _, H, Dh = B_Wq.shape
    seg = int(B_seg_len)
    assert B == 1 and B_x.shape == (B, S, D) and S % A_CHUNK == 0 and A_CHUNK % seg == 0
    assert D % LANES == 0 and D % A_HEADS == 0 and 4 * A_HEADS == LANES
    assert 2 * Dh == 3 * LANES and 2 * (seg + M) <= LANES and seg % 16 == 0 and M % 8 == 0
    n_t = D // LANES
    n_chunk = S // A_CHUNK
    assert H % 2 == 0 and (S // seg) % 2 == 0

    def head_major(w):
        return jnp.transpose(w, (1, 2, 0)).reshape(H * Dh, D)

    any_spec = pl.BlockSpec(memory_space=pl.ANY)
    out = pl.pallas_call(
        functools.partial(_kernel, seg=seg, b_heads=H, b_dh=Dh),
        in_specs=[any_spec] * 9,
        out_specs=any_spec,
        out_shape=jax.ShapeDtypeStruct((S, 2 * D), BF16),
        scratch_shapes=[
            pltpu.VMEM((S, D), BF16),
            pltpu.VMEM((3, D, D), BF16),
            pltpu.VMEM((D, D), BF16),
            pltpu.VMEM((3, D // 2, D), U32),
            pltpu.VMEM((D // 2, D), U32),
            pltpu.VMEM((n_t, D, LANES), F32),
            pltpu.VMEM((n_t, A_HALO + A_CHUNK, LANES), F32),
            pltpu.VMEM((n_t, A_HALO + A_CHUNK, LANES), F32),
            pltpu.VMEM((S, D), BF16),
            pltpu.VMEM((S, D), BF16),
            pltpu.VMEM((M, D), BF16),
            pltpu.VMEM((4, H * Dh, D), BF16),
            pltpu.VMEM((H // 2, D // 2, 6 * Dh), U32),
            pltpu.VMEM((H // 2, Dh, D), U32),
            pltpu.VMEM((S // seg * PRE, D), BF16),
            pltpu.VMEM((H // 2, S // seg * PRE, 2 * Dh), F32),
            pltpu.VMEM((B_UNROLL, seg + M, D), F32),
            pltpu.VMEM((S, D), BF16),
            pltpu.SemaphoreType.DMA((6 + n_chunk + H // 2 // P_UNROLL,)),
            pltpu.SemaphoreType.DMA((2,)),
        ],
        compiler_params=pltpu.CompilerParams(vmem_limit_bytes=112 * 1024 * 1024, flags=FLAGS),
        name="mbkern",
    )(
        A_x.reshape(S, D),
        A_wqkv,
        A_wo,
        B_x.reshape(S, D),
        B_mem0.reshape(M, D),
        head_major(B_Wq),
        head_major(B_Wk),
        head_major(B_Wv),
        B_Wo.reshape(H * Dh, D),
    )
    return out.reshape(B, S, 2 * D)
```

```python
import functools

import jax
import jax.numpy as jnp
from jax import lax
import jax.experimental.pallas as pl
import jax.experimental.pallas.tpu as pltpu

BF16 = jnp.bfloat16
F32 = jnp.float32
U32 = jnp.uint32
LANES = 128

_NN = (((1,), (0,)), ((), ()))
_NT = (((1,), (1,)), ((), ()))

A_HEADS = 32
A_WIN = 8
A_DIL = 2
A_HALO = 16
A_CHUNK = 256
A_ROWS = 64
A_D_OUT = 3
A_SUB = 8
MASK_VALUE = -1000000000.0

D_QK, D_PV, D_WO = 1, 3, 6
PRE = 8
B_UNROLL = 4
MEM_FIRST = True
P_STATIC = False
N_EARLY = 8
REGROUP_AT = (3, 4, 6, 7)
P_UNROLL = 2
FLAGS = None


def _dot(a, b, dims=_NN):
    return lax.dot_general(a, b, dims, preferred_element_type=F32)


def _kernel(
    ax_hbm, awqkv_hbm, awo_hbm, bx_hbm, mem_hbm, wq_hbm, wk_hbm, wv_hbm, wo_hbm,
    out_hbm,
    ax_v, aw_v, aw_p, atmp_v, ak_v, av_v, aout_v,
    bx_v, mem_v, wt_v, wqkv_v, wo_v, xpre_v, qpre_v, h_v, bout_v,
    sem_in, sem_out,
    *, seg, b_heads, b_dh,
):
    S, D = ax_hbm.shape
    n_t = D // LANES
    a_dh = D // A_HEADS
    n_chunk = S // A_CHUNK
    M = mem_hbm.shape[0]
    L = seg + M
    n_seg = S // seg
    n_pair = b_heads // 2
    PW = 2 * b_dh
    w_hbm = (wq_hbm, wk_hbm, wv_hbm, wo_hbm)

    n_early = N_EARLY
    n_group = n_pair // P_UNROLL
    n_late = (n_pair - n_early) // n_group
    S_AW, S_PRE, S_B, S_WQ = 0, 4, 5, 6
    S_AX = S_WQ + n_early
    S_W = S_AX + n_chunk

    def cp_aw(j):
        src = awo_hbm if j == 3 else awqkv_hbm.at[:, pl.ds(((j + 1) % 3) * D, D)]
        return pltpu.make_async_copy(src, aw_v.at[j], sem_in.at[S_AW + j])

    cp_pre = [
        pltpu.make_async_copy(
            bx_hbm.at[:, pl.ds(u * seg, PRE)], xpre_v.at[:, pl.ds(u * PRE, PRE)], sem_in.at[S_PRE])
        for u in range(2)]
    cp_b = [pltpu.make_async_copy(mem_hbm, mem_v, sem_in.at[S_B]),
            pltpu.make_async_copy(bx_hbm, bx_v, sem_in.at[S_B])]

    def cp_ax(c):
        rows = pl.ds(pl.multiple_of(c * A_CHUNK, A_CHUNK), A_CHUNK)
        return pltpu.make_async_copy(ax_hbm.at[rows], ax_v.at[rows], sem_in.at[S_AX + c])

    def pair_rows(i, n=1):
        return pl.ds(pl.multiple_of(i * PW, PW), n * PW)

    def cp_rows(m, rows, sem):
        return pltpu.make_async_copy(w_hbm[m].at[rows], wt_v.at[m, rows], sem_in.at[sem])

    def cp_wq(i):
        return cp_rows(0, pair_rows(i), S_WQ + i)

    def cp_w(g):
        return [cp_rows(0, pair_rows(n_early + g * n_late, n_late), S_W + g)] + [
            cp_rows(m, pair_rows(g * P_UNROLL, P_UNROLL), S_W + g) for m in (1, 2, 3)]

    def regroups(i):
        return [j for j in range(4) if REGROUP_AT[j] == i]

    for cp in cp_pre:
        cp.start()
    for i in range(n_early):
        for j in regroups(i):
            cp_aw(j).start()
        cp_wq(i).start()
    for c in range(n_chunk):
        cp_ax(c).start()
    for g in range(n_group):
        for cp in cp_w(g):
            cp.start()
    for cp in cp_b:
        cp.start()

    def regroup_rows(w):
        for t in range(n_t):
            atmp_v[t] = w[:, t * LANES:(t + 1) * LANES]
        return jnp.concatenate([
            jnp.concatenate(
                [atmp_v[t, pl.ds(d, A_HEADS, stride=a_dh), :] for t in range(n_t)], axis=1
            ).astype(BF16)
            for d in range(a_dh)
        ], axis=0)

    def regroup(j):
        w = aw_v[j].astype(F32)
        aw_p[j] = pltpu.bitcast(regroup_rows(w) if j == 3 else regroup_rows(w.T).T, U32)

    def leading_queries(i):
        x = xpre_v[...].reshape(n_seg * PRE, D)
        qpre_v[i] = _dot(x, wt_v[0, pair_rows(i), :], _NT)

    def transpose_w(i, m):
        wqkv_v[i, :, m * PW:(m + 1) * PW] = pltpu.bitcast(wt_v[m, pair_rows(i), :].T, U32)

    for cp in cp_pre:
        cp.wait()
    for i in range(n_early):
        for j in regroups(i):
            cp_aw(j).wait()
        cp_wq(i).wait()
        leading_queries(i)
        for j in regroups(i):
            regroup(j)
        transpose_w(i, 0)

    for buf in (ak_v, av_v):
        buf[:, 0:A_HALO, :] = jnp.zeros((n_t, A_HALO, LANES), F32)

    a_scale = float(a_dh) ** -0.5

    def a_chunk(c, carry):
        r0 = pl.multiple_of(c * A_CHUNK, A_CHUNK)

        cp_ax(c).wait()

        qs, os = {}, {}

        def project(i):
            x = ax_v[pl.ds(r0 + i * A_ROWS, A_ROWS), :]
            rows = pl.ds(A_HALO + i * A_ROWS, A_ROWS)
            for j, dst in enumerate((ak_v, av_v)):
                y = _dot(x, pltpu.bitcast(aw_p[j], BF16))
                for t in range(n_t):
                    dst[t, rows, :] = y[:, t * LANES:(t + 1) * LANES]
            if i == 0:
                for t in range(n_t):
                    row0 = jnp.broadcast_to(y[0:1, t * LANES:(t + 1) * LANES], (A_HALO, LANES))
                    av_v[t, 0:A_HALO, :] = jnp.where(c == 0, row0, av_v[t, 0:A_HALO, :])
            qs[i] = _dot(x, pltpu.bitcast(aw_p[2], BF16))

        def attend(i):
            q = qs.pop(i)
            blocks = []
            for b in range(A_ROWS // A_SUB):
                rq = b * A_SUB
                rb = i * A_ROWS + rq
                logits = []
                for w in range(A_WIN):
                    rows = pl.ds(A_HALO + rb - w * A_DIL, A_SUB)
                    acc = None
                    for t in range(n_t):
                        term = q[rq:rq + A_SUB, t * LANES:(t + 1) * LANES] * ak_v[t, rows, :]
                        acc = term if acc is None else acc + term
                    acc = acc + pltpu.roll(acc, 2 * A_HEADS, axis=1)
                    acc = acc + pltpu.roll(acc, A_HEADS, axis=1)
                    lg = acc * a_scale
                    if rb < w * A_DIL:
                        pos = r0 + rb + lax.broadcasted_iota(jnp.int32, (A_SUB, LANES), 0)
                        lg = jnp.where(pos >= w * A_DIL, lg, MASK_VALUE)
                    logits.append(lg)
                mx = functools.reduce(jnp.maximum, logits)
                es = [jnp.exp(lg - mx) for lg in logits]
                inv = 1.0 / functools.reduce(jnp.add, es)
                o_t = []
                for t in range(n_t):
                    acc = None
                    for w in range(A_WIN):
                        rows = pl.ds(A_HALO + rb - w * A_DIL, A_SUB)
                        term = es[w] * av_v[t, rows, :]
                        acc = term if acc is None else acc + term
                    o_t.append((acc * inv).astype(BF16))
                blocks.append(jnp.concatenate(o_t, axis=1))
            os[i] = jnp.concatenate(blocks, axis=0)

        def out_proj(i):
            y = _dot(os.pop(i), pltpu.bitcast(aw_p[3], BF16))
            aout_v[pl.ds(r0 + i * A_ROWS, A_ROWS), :] = y.astype(BF16)

        n_sub = A_CHUNK // A_ROWS
        for i in range(n_sub + A_D_OUT):
            if i < n_sub:
                project(i)
            if 0 <= i - 1 < n_sub:
                attend(i - 1)
            if 0 <= i - A_D_OUT < n_sub:
                out_proj(i - A_D_OUT)
        for buf in (ak_v, av_v):
            buf[:, 0:A_HALO, :] = buf[:, A_CHUNK:A_CHUNK + A_HALO, :]
        return carry

    lax.fori_loop(0, n_chunk, a_chunk, 0)

    cp_aout = pltpu.make_async_copy(aout_v, out_hbm.at[:, pl.ds(0, D)], sem_out.at[0])
    cp_aout.start()

    def prepare_pairs(g, carry):
        for cp in cp_w(g):
            cp.wait()
        for u in range(P_UNROLL):
            for n in range(-(-u * n_late // P_UNROLL), -(-(u + 1) * n_late // P_UNROLL)):
                i = n_early + g * n_late + n
                leading_queries(i)
                transpose_w(i, 0)
            i = g * P_UNROLL + u
            transpose_w(i, 1)
            transpose_w(i, 2)
            wo_v[i] = pltpu.bitcast(wt_v[3, pair_rows(i), :], U32)
        return carry

    lax.fori_loop(0, n_group, prepare_pairs, 0, unroll=P_STATIC)
    for cp in cp_b:
        cp.wait()

    b_scale = float(b_dh) ** -0.5
    h_v[0, seg:L, :] = mem_v[...].astype(F32)

    def b_segment(g, slot):
        s = g * B_UNROLL + slot
        r0 = pl.multiple_of(s * seg, seg)
        x = bx_v[g * (B_UNROLL // 2) + slot // 2, (slot % 2) * seg:(slot % 2 + 1) * seg, :]
        h_v[slot, 0:seg, :] = x.astype(F32)

        row = lax.broadcasted_iota(jnp.int32, (L, 2 * L), 0)
        col = lax.broadcasted_iota(jnp.int32, (L, 2 * L), 1)
        first = col < L
        key = jnp.where(first, col, col - L)
        mask = (row >= seg) | (key >= seg) | (key <= row)
        lo = lax.broadcasted_iota(jnp.int32, (L, LANES), 1) < b_dh - LANES

        def block_diag(t):
            z = jnp.zeros((L, LANES), F32)
            mid = t[:, LANES:2 * LANES]
            top = jnp.concatenate([t[:, 0:LANES], jnp.where(lo, mid, 0.0), z], axis=1)
            bot = jnp.concatenate([z, jnp.where(lo, 0.0, mid), t[:, 2 * LANES:]], axis=1)
            return jnp.concatenate([top, bot], axis=0).astype(BF16)

        q, kk, vv, p, o = {}, {}, {}, {}, {}
        acc = [None]

        def project(i):
            h = h_v[slot]
            w = pltpu.bitcast(wqkv_v[i], BF16)
            if i == 0 and slot > 0:
                k = functools.reduce(jnp.add, [
                    _dot(h[:, t * LANES:(t + 1) * LANES], w[t * LANES:(t + 1) * LANES, PW:2 * PW])
                    for t in range(n_t)])
            else:
                k = _dot(h, w[:, PW:2 * PW])
            kk[i] = block_diag(k)
            q[i] = jnp.concatenate([
                qpre_v[i, pl.ds(pl.multiple_of(s * PRE, PRE), PRE), :],
                _dot(h[PRE:], w[:, 0:PW])], axis=0)
            vv[i] = block_diag(_dot(h, w[:, 2 * PW:3 * PW]))

        def scores(i):
            sc = _dot(q.pop(i), kk.pop(i), _NT) * b_scale
            sc = jnp.where(mask, sc, MASK_VALUE)
            m0 = jnp.max(jnp.where(first, sc, -jnp.inf), axis=1, keepdims=True)
            m1 = jnp.max(jnp.where(first, -jnp.inf, sc), axis=1, keepdims=True)
            e = jnp.exp(sc - jnp.where(first, m0, m1))
            s0 = jnp.sum(jnp.where(first, e, 0.0), axis=1, keepdims=True)
            s1 = jnp.sum(jnp.where(first, 0.0, e), axis=1, keepdims=True)
            p[i] = e / jnp.where(first, s0, s1)

        def values(i):
            o[i] = _dot(p.pop(i), vv.pop(i))

        def out_proj(i):
            oi = o.pop(i)
            if MEM_FIRST:
                oi = jnp.concatenate([oi[seg:], oi[:seg]], axis=0)
            r = _dot(oi, pltpu.bitcast(wo_v[i], BF16))
            acc[0] = r if acc[0] is None else acc[0] + r

        done = 0
        i = 0
        while done < n_pair:
            if i < n_pair:
                project(i)
            if 0 <= i - D_QK < n_pair:
                scores(i - D_QK)
            if 0 <= i - D_PV < n_pair:
                values(i - D_PV)
            if i < n_pair:
                n = 1 if i >= D_WO else 0
            else:
                left = n_pair + D_PV - i
                ready = min(n_pair, i - D_PV) - done
                n = min(-(-(n_pair - 1 - done) // left), ready) if left > 0 else n_pair - done
            for _ in range(n):
                out_proj(done)
                done += 1
            i += 1

        new_mem, res = (acc[0][:M], acc[0][M:]) if MEM_FIRST else (acc[0][seg:], acc[0][:seg])
        h_v[(slot + 1) % B_UNROLL, seg:L, :] = new_mem
        rows = pl.ds(r0, seg)
        bout_v[rows, :] = res.astype(BF16)
        pltpu.make_async_copy(
            bout_v.at[rows], out_hbm.at[rows, pl.ds(D, D)], sem_out.at[1]).start()

    def b_step(g, carry):
        for u in range(B_UNROLL):
            b_segment(g, u)
        return carry

    lax.fori_loop(0, n_seg // B_UNROLL, b_step, 0)

    cp_aout.wait()
    pltpu.make_async_copy(bout_v, out_hbm.at[:, pl.ds(D, D)], sem_out.at[1]).wait()


@functools.partial(jax.jit, static_argnames=("B_seg_len",))
def pallas_concat_heads__sliding_local_dilated__memory_aug_recurrent_mem_tr__prompt_kernel(
    A_x: jax.Array,
    A_wqkv: jax.Array,
    A_wo: jax.Array,
    B_x: jax.Array,
    B_mem0: jax.Array,
    B_Wq: jax.Array,
    B_Wk: jax.Array,
    B_Wv: jax.Array,
    B_Wo: jax.Array,
    B_seg_len: int,
):
    B, S, D = A_x.shape
    M = B_mem0.shape[1]
    _, H, Dh = B_Wq.shape
    seg = int(B_seg_len)
    assert B == 1 and B_x.shape == (B, S, D) and S % A_CHUNK == 0 and A_CHUNK % seg == 0
    assert D % LANES == 0 and D % A_HEADS == 0 and 4 * A_HEADS == LANES
    assert 2 * Dh == 3 * LANES and 2 * (seg + M) <= LANES and seg % 16 == 0 and M % 8 == 0
    n_t = D // LANES
    n_chunk = S // A_CHUNK
    assert H % 2 == 0 and (S // seg) % 2 == 0

    def head_major(w):
        return jnp.transpose(w, (1, 2, 0)).reshape(H * Dh, D)

    any_spec = pl.BlockSpec(memory_space=pl.ANY)
    out = pl.pallas_call(
        functools.partial(_kernel, seg=seg, b_heads=H, b_dh=Dh),
        in_specs=[any_spec] * 9,
        out_specs=any_spec,
        out_shape=jax.ShapeDtypeStruct((S, 2 * D), BF16),
        scratch_shapes=[
            pltpu.VMEM((S, D), BF16),
            pltpu.VMEM((4, D, D), BF16),
            pltpu.VMEM((4, D // 2, D), U32),
            pltpu.VMEM((n_t, D, LANES), F32),
            pltpu.VMEM((n_t, A_HALO + A_CHUNK, LANES), F32),
            pltpu.VMEM((n_t, A_HALO + A_CHUNK, LANES), F32),
            pltpu.VMEM((S, D), BF16),
            pltpu.VMEM((S // (2 * seg), 2 * seg, D), BF16),
            pltpu.VMEM((M, D), BF16),
            pltpu.VMEM((4, H * Dh, D), BF16),
            pltpu.VMEM((H // 2, D // 2, 6 * Dh), U32),
            pltpu.VMEM((H // 2, Dh, D), U32),
            pltpu.VMEM((S // (2 * seg), 2 * PRE, D), BF16),
            pltpu.VMEM((H // 2, S // seg * PRE, 2 * Dh), F32),
            pltpu.VMEM((B_UNROLL, seg + M, D), F32),
            pltpu.VMEM((S, D), BF16),
            pltpu.SemaphoreType.DMA((6 + N_EARLY + n_chunk + H // 2 // P_UNROLL,)),
            pltpu.SemaphoreType.DMA((2,)),
        ],
        compiler_params=pltpu.CompilerParams(vmem_limit_bytes=112 * 1024 * 1024, flags=FLAGS),
        name="mbkern",
    )(
        A_x.reshape(S, D),
        A_wqkv,
        A_wo,
        B_x.reshape(S // (2 * seg), 2 * seg, D),
        B_mem0.reshape(M, D),
        head_major(B_Wq),
        head_major(B_Wk),
        head_major(B_Wv),
        B_Wo.reshape(H * Dh, D),
    )
    return out.reshape(B, S, 2 * D)
```

```python
import functools

import jax
import jax.numpy as jnp
from jax import lax
import jax.experimental.pallas as pl
import jax.experimental.pallas.tpu as pltpu

BF16 = jnp.bfloat16
F32 = jnp.float32
U32 = jnp.uint32
LANES = 128

_NN = (((1,), (0,)), ((), ()))
_NT = (((1,), (1,)), ((), ()))

A_HEADS = 32
A_WIN = 8
A_DIL = 2
A_HALO = 16
A_CHUNK = 256
A_ROWS = 64
A_D_OUT = 3
A_SUB = 8
MASK_VALUE = -1000000000.0

D_QK, D_PV, D_WO = 1, 3, 6
PRE = 8
B_UNROLL = 4
MEM_FIRST = True
N_FIRST = 2
N_REGROUP = 2
N_GROUP = 2
Q_ROWS = 128
FLAGS = None


def _dot(a, b, dims=_NN):
    return lax.dot_general(a, b, dims, preferred_element_type=F32)


def _kernel(
    ax_hbm, awqkv_hbm, awo_hbm, bx_hbm, mem_hbm, wq_hbm, wk_hbm, wv_hbm, wo_hbm,
    out_hbm,
    ax_v, aw_v, aw_p, atmp_v, ak_v, av_v, aout_v,
    bx_v, mem_v, wt_v, wqkv_v, wo_v, xpre_v, qpre_v, h_v, bout_v,
    sem_in, sem_out,
    *, seg, b_heads, b_dh,
):
    S, D = ax_hbm.shape
    n_t = D // LANES
    a_dh = D // A_HEADS
    n_chunk = S // A_CHUNK
    M = mem_hbm.shape[0]
    L = seg + M
    n_seg = S // seg
    n_pair = b_heads // 2
    PW = 2 * b_dh
    w_hbm = (wq_hbm, wk_hbm, wv_hbm)

    n_early = N_FIRST + 3 * N_REGROUP
    n_late = (n_pair - n_early) // N_GROUP
    ppg = n_pair // N_GROUP
    S_B, S_AWO, S_FIRST = 0, 1, 2
    S_REGROUP = S_FIRST + N_FIRST
    S_CHUNK = S_REGROUP + 3
    S_GROUP = S_CHUNK + n_chunk

    def pair_rows(i, n=1):
        return pl.ds(pl.multiple_of(i * PW, PW), n * PW)

    def cp_rows(m, rows, sem):
        return pltpu.make_async_copy(w_hbm[m].at[rows], wt_v.at[m, rows], sem)

    def cp_first(i):
        sem = sem_in.at[S_FIRST + i]
        cps = [cp_rows(0, pair_rows(i), sem)]
        if i == 0:
            cps += [
                pltpu.make_async_copy(
                    bx_hbm.at[:, pl.ds(u * seg, PRE)], xpre_v.at[:, pl.ds(u * PRE, PRE)], sem)
                for u in range(2)]
        return cps

    def cp_regroup(j):
        sem = sem_in.at[S_REGROUP + j]
        cols = pl.ds(pl.multiple_of(j * D, LANES), D)
        return [
            pltpu.make_async_copy(awqkv_hbm.at[:, cols], aw_v.at[j], sem),
            cp_rows(0, pair_rows(N_FIRST + j * N_REGROUP, N_REGROUP), sem),
        ]

    cp_awo = pltpu.make_async_copy(awo_hbm, aw_v.at[3], sem_in.at[S_AWO])

    def cp_chunk(c):
        rows = pl.ds(pl.multiple_of(c * A_CHUNK, A_CHUNK), A_CHUNK)
        return pltpu.make_async_copy(ax_hbm.at[rows], ax_v.at[rows], sem_in.at[S_CHUNK + c])

    def cp_group(g):
        sem = sem_in.at[S_GROUP + g]
        return [
            cp_rows(0, pair_rows(n_early + g * n_late, n_late), sem),
            cp_rows(1, pair_rows(g * ppg, ppg), sem),
            cp_rows(2, pair_rows(g * ppg, ppg), sem),
        ]

    cp_b = [
        pltpu.make_async_copy(wo_hbm.at[:, pl.ds(t * LANES, LANES)], wo_v.at[t], sem_in.at[S_B])
        for t in range(n_t)
    ] + [
        pltpu.make_async_copy(mem_hbm, mem_v, sem_in.at[S_B]),
        pltpu.make_async_copy(bx_hbm, bx_v, sem_in.at[S_B]),
    ]

    for i in range(N_FIRST):
        for cp in cp_first(i):
            cp.start()
    for j in range(3):
        for cp in cp_regroup(j):
            cp.start()
    cp_awo.start()
    for c in range(n_chunk):
        cp_chunk(c).start()
    for g in range(N_GROUP):
        for cp in cp_group(g):
            cp.start()
    for cp in cp_b:
        cp.start()

    def regroup_rows(w):
        for t in range(n_t):
            atmp_v[t] = w[:, t * LANES:(t + 1) * LANES]
        return jnp.concatenate([
            jnp.concatenate(
                [atmp_v[t, pl.ds(d, A_HEADS, stride=a_dh), :] for t in range(n_t)], axis=1
            ).astype(BF16)
            for d in range(a_dh)
        ], axis=0)

    def leading_queries(i):
        n = Q_ROWS // (2 * PRE)
        for b in range(n_seg * PRE // Q_ROWS):
            x = xpre_v[b * n:(b + 1) * n].reshape(Q_ROWS, D)
            qpre_v[i, b * Q_ROWS:(b + 1) * Q_ROWS, :] = _dot(x, wt_v[0, pair_rows(i), :], _NT)

    def transpose_w(i, m):
        wqkv_v[i, :, m * PW:(m + 1) * PW] = pltpu.bitcast(wt_v[m, pair_rows(i), :].T, U32)

    for i in range(N_FIRST):
        for cp in cp_first(i):
            cp.wait()
        leading_queries(i)
        transpose_w(i, 0)

    def regroup(j, carry):
        for cp in cp_regroup(j):
            cp.wait()
        aw_p[j] = pltpu.bitcast(regroup_rows(aw_v[j].astype(F32).T).T, U32)
        for n in range(N_REGROUP):
            leading_queries(N_FIRST + j * N_REGROUP + n)
            transpose_w(N_FIRST + j * N_REGROUP + n, 0)
        return carry

    lax.fori_loop(0, 3, regroup, 0)
    cp_awo.wait()
    aw_p[3] = pltpu.bitcast(regroup_rows(aw_v[3].astype(F32)), U32)

    for buf in (ak_v, av_v):
        buf[:, 0:A_HALO, :] = jnp.zeros((n_t, A_HALO, LANES), F32)

    a_scale = float(a_dh) ** -0.5

    def a_chunk(c, carry):
        r0 = pl.multiple_of(c * A_CHUNK, A_CHUNK)

        cp_chunk(c).wait()

        qs, os = {}, {}

        def project(i):
            x = ax_v[pl.ds(r0 + i * A_ROWS, A_ROWS), :]
            rows = pl.ds(A_HALO + i * A_ROWS, A_ROWS)
            for j, dst in ((1, ak_v), (2, av_v)):
                y = _dot(x, pltpu.bitcast(aw_p[j], BF16))
                for t in range(n_t):
                    dst[t, rows, :] = y[:, t * LANES:(t + 1) * LANES]
            if i == 0:
                for t in range(n_t):
                    row0 = jnp.broadcast_to(y[0:1, t * LANES:(t + 1) * LANES], (A_HALO, LANES))
                    av_v[t, 0:A_HALO, :] = jnp.where(c == 0, row0, av_v[t, 0:A_HALO, :])
            qs[i] = _dot(x, pltpu.bitcast(aw_p[0], BF16))

        def attend(i):
            q = qs.pop(i)
            blocks = []
            for b in range(A_ROWS // A_SUB):
                rq = b * A_SUB
                rb = i * A_ROWS + rq
                logits = []
                for w in range(A_WIN):
                    rows = pl.ds(A_HALO + rb - w * A_DIL, A_SUB)
                    acc = None
                    for t in range(n_t):
                        term = q[rq:rq + A_SUB, t * LANES:(t + 1) * LANES] * ak_v[t, rows, :]
                        acc = term if acc is None else acc + term
                    acc = acc + pltpu.roll(acc, 2 * A_HEADS, axis=1)
                    acc = acc + pltpu.roll(acc, A_HEADS, axis=1)
                    lg = acc * a_scale
                    if rb < w * A_DIL:
                        pos = r0 + rb + lax.broadcasted_iota(jnp.int32, (A_SUB, LANES), 0)
                        lg = jnp.where(pos >= w * A_DIL, lg, MASK_VALUE)
                    logits.append(lg)
                mx = functools.reduce(jnp.maximum, logits)
                es = [jnp.exp(lg - mx) for lg in logits]
                inv = 1.0 / functools.reduce(jnp.add, es)
                o_t = []
                for t in range(n_t):
                    acc = None
                    for w in range(A_WIN):
                        rows = pl.ds(A_HALO + rb - w * A_DIL, A_SUB)
                        term = es[w] * av_v[t, rows, :]
                        acc = term if acc is None else acc + term
                    o_t.append((acc * inv).astype(BF16))
                blocks.append(jnp.concatenate(o_t, axis=1))
            os[i] = jnp.concatenate(blocks, axis=0)

        def out_proj(i):
            y = _dot(os.pop(i), pltpu.bitcast(aw_p[3], BF16))
            aout_v[pl.ds(r0 + i * A_ROWS, A_ROWS), :] = y.astype(BF16)

        n_sub = A_CHUNK // A_ROWS
        for i in range(n_sub + A_D_OUT):
            if i < n_sub:
                project(i)
            if 0 <= i - 1 < n_sub:
                attend(i - 1)
            if 0 <= i - A_D_OUT < n_sub:
                out_proj(i - A_D_OUT)
        for buf in (ak_v, av_v):
            buf[:, 0:A_HALO, :] = buf[:, A_CHUNK:A_CHUNK + A_HALO, :]
        return carry

    lax.fori_loop(0, n_chunk, a_chunk, 0)

    cp_aout = pltpu.make_async_copy(aout_v, out_hbm.at[:, pl.ds(0, D)], sem_out.at[0])
    cp_aout.start()

    def prepare_group(g, carry):
        for cp in cp_group(g):
            cp.wait()
        for n in range(n_late):
            leading_queries(n_early + g * n_late + n)
            transpose_w(n_early + g * n_late + n, 0)
        for n in range(ppg):
            transpose_w(g * ppg + n, 1)
            transpose_w(g * ppg + n, 2)
        return carry

    lax.fori_loop(0, N_GROUP, prepare_group, 0)
    for cp in cp_b:
        cp.wait()

    b_scale = float(b_dh) ** -0.5
    wo_w = wo_v.bitcast(U32)
    h_v[0, seg:L, :] = mem_v[...].astype(F32)

    def b_segment(g, slot):
        s = g * B_UNROLL + slot
        r0 = pl.multiple_of(s * seg, seg)
        x = bx_v[g * (B_UNROLL // 2) + slot // 2, (slot % 2) * seg:(slot % 2 + 1) * seg, :]
        h_v[slot, 0:seg, :] = x.astype(F32)

        row = lax.broadcasted_iota(jnp.int32, (L, 2 * L), 0)
        col = lax.broadcasted_iota(jnp.int32, (L, 2 * L), 1)
        first = col < L
        key = jnp.where(first, col, col - L)
        mask = (row >= seg) | (key >= seg) | (key <= row)
        lo = lax.broadcasted_iota(jnp.int32, (L, LANES), 1) < b_dh - LANES

        def block_diag(t):
            z = jnp.zeros((L, LANES), F32)
            mid = t[:, LANES:2 * LANES]
            top = jnp.concatenate([t[:, 0:LANES], jnp.where(lo, mid, 0.0), z], axis=1)
            bot = jnp.concatenate([z, jnp.where(lo, 0.0, mid), t[:, 2 * LANES:]], axis=1)
            return jnp.concatenate([top, bot], axis=0).astype(BF16)

        q, kk, vv, p, o = {}, {}, {}, {}, {}
        acc = [None]

        def project(i):
            h = h_v[slot]
            w = pltpu.bitcast(wqkv_v[i], BF16)
            if i == 0 and slot > 0:
                k = functools.reduce(jnp.add, [
                    _dot(h[:, t * LANES:(t + 1) * LANES], w[t * LANES:(t + 1) * LANES, PW:2 * PW])
                    for t in range(n_t)])
            else:
                k = _dot(h, w[:, PW:2 * PW])
            kk[i] = block_diag(k)
            q[i] = jnp.concatenate([
                qpre_v[i, pl.ds(pl.multiple_of(s * PRE, PRE), PRE), :],
                _dot(h[PRE:], w[:, 0:PW])], axis=0)
            vv[i] = block_diag(_dot(h, w[:, 2 * PW:3 * PW]))

        def scores(i):
            sc = _dot(q.pop(i), kk.pop(i), _NT) * b_scale
            sc = jnp.where(mask, sc, MASK_VALUE)
            m0 = jnp.max(jnp.where(first, sc, -jnp.inf), axis=1, keepdims=True)
            m1 = jnp.max(jnp.where(first, -jnp.inf, sc), axis=1, keepdims=True)
            e = jnp.exp(sc - jnp.where(first, m0, m1))
            s0 = jnp.sum(jnp.where(first, e, 0.0), axis=1, keepdims=True)
            s1 = jnp.sum(jnp.where(first, 0.0, e), axis=1, keepdims=True)
            p[i] = e / jnp.where(first, s0, s1)

        def values(i):
            o[i] = _dot(p.pop(i), vv.pop(i))

        def out_proj(i):
            oi = o.pop(i)
            if MEM_FIRST:
                oi = jnp.concatenate([oi[seg:], oi[:seg]], axis=0)
            rows = slice(i * PW // 2, (i + 1) * PW // 2)
            r = _dot(oi, jnp.concatenate(
                [pltpu.bitcast(wo_w[t, rows, :], BF16) for t in range(n_t)], axis=1))
            acc[0] = r if acc[0] is None else acc[0] + r

        done = 0
        i = 0
        while done < n_pair:
            if i < n_pair:
                project(i)
            if 0 <= i - D_QK < n_pair:
                scores(i - D_QK)
            if 0 <= i - D_PV < n_pair:
                values(i - D_PV)
            if i < n_pair:
                n = 1 if i >= D_WO else 0
            else:
                left = n_pair + D_PV - i
                ready = min(n_pair, i - D_PV) - done
                n = min(-(-(n_pair - 1 - done) // left), ready) if left > 0 else n_pair - done
            for _ in range(n):
                out_proj(done)
                done += 1
            i += 1

        new_mem, res = (acc[0][:M], acc[0][M:]) if MEM_FIRST else (acc[0][seg:], acc[0][:seg])
        h_v[(slot + 1) % B_UNROLL, seg:L, :] = new_mem
        rows = pl.ds(r0, seg)
        bout_v[rows, :] = res.astype(BF16)
        pltpu.make_async_copy(
            bout_v.at[rows], out_hbm.at[rows, pl.ds(D, D)], sem_out.at[1]).start()

    def b_step(g, carry):
        for u in range(B_UNROLL):
            b_segment(g, u)
        return carry

    lax.fori_loop(0, n_seg // B_UNROLL, b_step, 0)

    cp_aout.wait()
    pltpu.make_async_copy(bout_v, out_hbm.at[:, pl.ds(D, D)], sem_out.at[1]).wait()


@functools.partial(jax.jit, static_argnames=("B_seg_len",))
def pallas_concat_heads__sliding_local_dilated__memory_aug_recurrent_mem_tr__prompt_kernel(
    A_x: jax.Array,
    A_wqkv: jax.Array,
    A_wo: jax.Array,
    B_x: jax.Array,
    B_mem0: jax.Array,
    B_Wq: jax.Array,
    B_Wk: jax.Array,
    B_Wv: jax.Array,
    B_Wo: jax.Array,
    B_seg_len: int,
):
    B, S, D = A_x.shape
    M = B_mem0.shape[1]
    _, H, Dh = B_Wq.shape
    seg = int(B_seg_len)
    assert B == 1 and B_x.shape == (B, S, D) and S % A_CHUNK == 0 and A_CHUNK % seg == 0
    assert D % LANES == 0 and D % A_HEADS == 0 and 4 * A_HEADS == LANES
    assert 2 * Dh == 3 * LANES and 2 * (seg + M) <= LANES and seg % 16 == 0 and M % 8 == 0
    n_t = D // LANES
    n_chunk = S // A_CHUNK
    assert H % 2 == 0 and (S // seg) % 2 == 0

    def head_major(w):
        return jnp.transpose(w, (1, 2, 0)).reshape(H * Dh, D)

    any_spec = pl.BlockSpec(memory_space=pl.ANY)
    out = pl.pallas_call(
        functools.partial(_kernel, seg=seg, b_heads=H, b_dh=Dh),
        in_specs=[any_spec] * 9,
        out_specs=any_spec,
        out_shape=jax.ShapeDtypeStruct((S, 2 * D), BF16),
        scratch_shapes=[
            pltpu.VMEM((S, D), BF16),
            pltpu.VMEM((4, D, D), BF16),
            pltpu.VMEM((4, D // 2, D), U32),
            pltpu.VMEM((n_t, D, LANES), F32),
            pltpu.VMEM((n_t, A_HALO + A_CHUNK, LANES), F32),
            pltpu.VMEM((n_t, A_HALO + A_CHUNK, LANES), F32),
            pltpu.VMEM((S, D), BF16),
            pltpu.VMEM((S // (2 * seg), 2 * seg, D), BF16),
            pltpu.VMEM((M, D), BF16),
            pltpu.VMEM((3, H * Dh, D), BF16),
            pltpu.VMEM((H // 2, D // 2, 6 * Dh), U32),
            pltpu.VMEM((n_t, H * Dh, LANES), BF16),
            pltpu.VMEM((S // (2 * seg), 2 * PRE, D), BF16),
            pltpu.VMEM((H // 2, S // seg * PRE, 2 * Dh), F32),
            pltpu.VMEM((B_UNROLL, seg + M, D), F32),
            pltpu.VMEM((S, D), BF16),
            pltpu.SemaphoreType.DMA((5 + N_FIRST + n_chunk + N_GROUP,)),
            pltpu.SemaphoreType.DMA((2,)),
        ],
        compiler_params=pltpu.CompilerParams(vmem_limit_bytes=112 * 1024 * 1024, flags=FLAGS),
        name="mbkern",
    )(
        A_x.reshape(S, D),
        A_wqkv,
        A_wo,
        B_x.reshape(S // (2 * seg), 2 * seg, D),
        B_mem0.reshape(M, D),
        head_major(B_Wq),
        head_major(B_Wk),
        head_major(B_Wv),
        B_Wo.reshape(H * Dh, D),
    )
    return out.reshape(B, S, 2 * D)
```

```python
import functools

import jax
import jax.numpy as jnp
from jax import lax
import jax.experimental.pallas as pl
import jax.experimental.pallas.tpu as pltpu

BF16 = jnp.bfloat16
F32 = jnp.float32
U32 = jnp.uint32
LANES = 128
MASK_VALUE = -1000000000.0

_NN = (((1,), (0,)), ((), ()))
_NT = (((1,), (1,)), ((), ()))

A_HEADS = 32
A_WIN = 8
A_DIL = 2

A_HALO = 16
A_CHUNK = 256
A_ROWS = 64
A_SUB = 8
A_D_OUT = 3

B_UNROLL = 4
D_QK, D_PV, D_WO = 1, 3, 6
PRE = 8
PRE_ROWS = 128
N_FIRST = 2
N_REGROUP = 2
N_GROUP = 2


def _dot(a, b, dims=_NN):
    return lax.dot_general(a, b, dims, preferred_element_type=F32)


def _tile(x, t):
    return x[:, t * LANES:(t + 1) * LANES]


def _kernel(
    ax_hbm, awqkv_hbm, awo_hbm, bx_hbm, mem_hbm, wq_hbm, wk_hbm, wv_hbm, wo_hbm,
    out_hbm,
    ax_v, aw_v, aw_p, atmp_v, ak_v, av_v, aout_v,
    bx_v, mem_v, wt_v, wqkv_v, wo_v, xpre_v, qpre_v, h_v, bout_v,
    sem_in, sem_out,
    *, seg, b_heads, b_dh,
):
    S, D = ax_hbm.shape
    n_t = D // LANES
    a_dh = D // A_HEADS
    n_chunk = S // A_CHUNK
    M = mem_hbm.shape[0]
    L = seg + M
    n_seg = S // seg
    n_pair = b_heads // 2
    PW = 2 * b_dh
    wt_hbm = (wq_hbm, wk_hbm, wv_hbm)

    n_early = N_FIRST + 3 * N_REGROUP
    n_late = (n_pair - n_early) // N_GROUP
    ppg = n_pair // N_GROUP
    S_B, S_AWO, S_FIRST = 0, 1, 2
    S_REGROUP = S_FIRST + N_FIRST
    S_CHUNK = S_REGROUP + 3
    S_GROUP = S_CHUNK + n_chunk

    def pair_rows(i, n=1):
        return pl.ds(pl.multiple_of(i * PW, PW), n * PW)

    def cp_wt(m, rows, sem):
        return pltpu.make_async_copy(wt_hbm[m].at[rows], wt_v.at[m, rows], sem)

    def cp_first(i):
        sem = sem_in.at[S_FIRST + i]
        cps = [cp_wt(0, pair_rows(i), sem)]
        if i == 0:
            cps += [
                pltpu.make_async_copy(
                    bx_hbm.at[:, pl.ds(u * seg, PRE)], xpre_v.at[:, pl.ds(u * PRE, PRE)], sem)
                for u in range(2)]
        return cps

    def cp_regroup(j):
        sem = sem_in.at[S_REGROUP + j]
        cols = pl.ds(pl.multiple_of(j * D, LANES), D)
        return [
            pltpu.make_async_copy(awqkv_hbm.at[:, cols], aw_v.at[j], sem),
            cp_wt(0, pair_rows(N_FIRST + j * N_REGROUP, N_REGROUP), sem),
        ]

    cp_awo = pltpu.make_async_copy(awo_hbm, aw_v.at[3], sem_in.at[S_AWO])

    def cp_chunk(c):
        rows = pl.ds(pl.multiple_of(c * A_CHUNK, A_CHUNK), A_CHUNK)
        return pltpu.make_async_copy(ax_hbm.at[rows], ax_v.at[rows], sem_in.at[S_CHUNK + c])

    def cp_group(g):
        sem = sem_in.at[S_GROUP + g]
        return [
            cp_wt(0, pair_rows(n_early + g * n_late, n_late), sem),
            cp_wt(1, pair_rows(g * ppg, ppg), sem),
            cp_wt(2, pair_rows(g * ppg, ppg), sem),
        ]

    cp_b = [
        pltpu.make_async_copy(wo_hbm, wo_v, sem_in.at[S_B]),
        pltpu.make_async_copy(mem_hbm, mem_v, sem_in.at[S_B]),
        pltpu.make_async_copy(bx_hbm, bx_v, sem_in.at[S_B]),
    ]

    for i in range(N_FIRST):
        for cp in cp_first(i):
            cp.start()
    for j in range(3):
        for cp in cp_regroup(j):
            cp.start()
    cp_awo.start()
    for c in range(n_chunk):
        cp_chunk(c).start()
    for g in range(N_GROUP):
        for cp in cp_group(g):
            cp.start()
    for cp in cp_b:
        cp.start()

    atmp_v[:, D:, :] = jnp.zeros((n_t, atmp_v.shape[1] - D, LANES), F32)

    def regroup_rows(w):
        for t in range(n_t):
            atmp_v[t, 0:D, :] = _tile(w, t)
        return jnp.concatenate([
            jnp.concatenate(
                [atmp_v[t, pl.ds(d, A_HEADS, stride=a_dh), :] for t in range(n_t)], axis=1
            ).astype(BF16)
            for d in range(a_dh)
        ], axis=0)

    def leading_queries(i):
        n = PRE_ROWS // (2 * PRE)
        for b in range(n_seg * PRE // PRE_ROWS):
            x = xpre_v[b * n:(b + 1) * n].reshape(PRE_ROWS, D)
            qpre_v[i, b * PRE_ROWS:(b + 1) * PRE_ROWS, :] = _dot(
                x, wt_v[0, pair_rows(i), :], _NT)

    def transpose_w(i, m):
        wqkv_v[i, :, m * PW:(m + 1) * PW] = pltpu.bitcast(wt_v[m, pair_rows(i), :].T, U32)

    for i in range(N_FIRST):
        for cp in cp_first(i):
            cp.wait()
        leading_queries(i)
        transpose_w(i, 0)

    def regroup(j, carry):
        for cp in cp_regroup(j):
            cp.wait()
        aw_p[j] = pltpu.bitcast(regroup_rows(aw_v[j].astype(F32).T).T, U32)
        for n in range(N_REGROUP):
            leading_queries(N_FIRST + j * N_REGROUP + n)
            transpose_w(N_FIRST + j * N_REGROUP + n, 0)
        return carry

    lax.fori_loop(0, 3, regroup, 0)
    cp_awo.wait()
    aw_p[3] = pltpu.bitcast(regroup_rows(aw_v[3].astype(F32)), U32)

    a_scale = float(a_dh) ** -0.5
    for buf in (ak_v, av_v):
        buf[:, 0:A_HALO, :] = jnp.zeros((n_t, A_HALO, LANES), F32)

    def a_chunk(c, carry):
        r0 = pl.multiple_of(c * A_CHUNK, A_CHUNK)
        cp_chunk(c).wait()
        qs, outs = {}, {}

        def project(i):
            x = ax_v[pl.ds(r0 + i * A_ROWS, A_ROWS), :]
            rows = pl.ds(A_HALO + i * A_ROWS, A_ROWS)
            v = _dot(x, pltpu.bitcast(aw_p[2], BF16))
            for t in range(n_t):
                av_v[t, rows, :] = _tile(v, t)
            if i == 0:
                for t in range(n_t):
                    row0 = jnp.broadcast_to(_tile(v, t)[0:1], (A_HALO, LANES))
                    av_v[t, 0:A_HALO, :] = jnp.where(c == 0, row0, av_v[t, 0:A_HALO, :])
            k = _dot(x, pltpu.bitcast(aw_p[1], BF16))
            for t in range(n_t):
                ak_v[t, rows, :] = _tile(k, t)
            qs[i] = _dot(x, pltpu.bitcast(aw_p[0], BF16))

        def attend(i):
            q = qs.pop(i)
            blocks = []
            for rq in range(0, A_ROWS, A_SUB):
                rb = i * A_ROWS + rq
                window = [pl.ds(A_HALO + rb - w * A_DIL, A_SUB) for w in range(A_WIN)]
                logits = []
                for w, rows in enumerate(window):
                    acc = functools.reduce(jnp.add, [
                        _tile(q, t)[rq:rq + A_SUB] * ak_v[t, rows, :] for t in range(n_t)])
                    acc = acc + pltpu.roll(acc, 2 * A_HEADS, axis=1)
                    acc = acc + pltpu.roll(acc, A_HEADS, axis=1)
                    lg = acc * a_scale
                    if rb < w * A_DIL:
                        pos = r0 + rb + lax.broadcasted_iota(jnp.int32, (A_SUB, LANES), 0)
                        lg = jnp.where(pos >= w * A_DIL, lg, MASK_VALUE)
                    logits.append(lg)
                mx = functools.reduce(jnp.maximum, logits)
                es = [jnp.exp(lg - mx) for lg in logits]
                inv = 1.0 / functools.reduce(jnp.add, es)
                blocks.append(jnp.concatenate([
                    (functools.reduce(
                        jnp.add, [e * av_v[t, rows, :] for e, rows in zip(es, window)]
                    ) * inv).astype(BF16)
                    for t in range(n_t)], axis=1))
            outs[i] = jnp.concatenate(blocks, axis=0)

        def out_proj(i):
            y = _dot(outs.pop(i), pltpu.bitcast(aw_p[3], BF16))
            aout_v[pl.ds(r0 + i * A_ROWS, A_ROWS), :] = y.astype(BF16)

        n_sub = A_CHUNK // A_ROWS
        for i in range(n_sub + A_D_OUT):
            if i < n_sub:
                project(i)
            if 0 <= i - 1 < n_sub:
                attend(i - 1)
            if 0 <= i - A_D_OUT < n_sub:
                out_proj(i - A_D_OUT)
        for buf in (ak_v, av_v):
            buf[:, 0:A_HALO, :] = buf[:, A_CHUNK:A_CHUNK + A_HALO, :]
        return carry

    lax.fori_loop(0, n_chunk, a_chunk, 0)

    cp_aout = pltpu.make_async_copy(aout_v, out_hbm.at[:, pl.ds(0, D)], sem_out.at[0])
    cp_aout.start()

    def prepare_group(g, carry):
        for cp in cp_group(g):
            cp.wait()
        for n in range(n_late):
            leading_queries(n_early + g * n_late + n)
            transpose_w(n_early + g * n_late + n, 0)
        for n in range(ppg):
            transpose_w(g * ppg + n, 1)
            transpose_w(g * ppg + n, 2)
        return carry

    lax.fori_loop(0, N_GROUP, prepare_group, 0)
    for cp in cp_b:
        cp.wait()

    b_scale = float(b_dh) ** -0.5
    h_v[0, seg:L, :] = mem_v[...].astype(F32)

    def b_segment(g, slot):
        s = g * B_UNROLL + slot
        x = bx_v[g * (B_UNROLL // 2) + slot // 2, (slot % 2) * seg:(slot % 2 + 1) * seg, :]
        h_v[slot, 0:seg, :] = x.astype(F32)

        row = lax.broadcasted_iota(jnp.int32, (L, 2 * L), 0)
        col = lax.broadcasted_iota(jnp.int32, (L, 2 * L), 1)
        first = col < L
        key = jnp.where(first, col, col - L)
        mask = (row >= seg) | (key >= seg) | (key <= row)
        lo = lax.broadcasted_iota(jnp.int32, (L, LANES), 1) < b_dh - LANES

        def block_diag(t):
            z = jnp.zeros((L, LANES), F32)
            top = jnp.concatenate([_tile(t, 0), jnp.where(lo, _tile(t, 1), 0.0), z], axis=1)
            bot = jnp.concatenate([z, jnp.where(lo, 0.0, _tile(t, 1)), _tile(t, 2)], axis=1)
            return jnp.concatenate([top, bot], axis=0).astype(BF16)

        q, kk, vv, p, o = {}, {}, {}, {}, {}
        acc = [None]

        def project(i):
            h = h_v[slot]
            w = pltpu.bitcast(wqkv_v[i], BF16)
            if i == 0 and slot > 0:
                k = functools.reduce(jnp.add, [
                    _dot(_tile(h, t), w[t * LANES:(t + 1) * LANES, PW:2 * PW])
                    for t in range(n_t)])
            else:
                k = _dot(h, w[:, PW:2 * PW])
            kk[i] = block_diag(k)
            q[i] = jnp.concatenate([
                qpre_v[i, pl.ds(pl.multiple_of(s * PRE, PRE), PRE), :],
                _dot(h[PRE:], w[:, 0:PW])], axis=0)
            vv[i] = block_diag(_dot(h, w[:, 2 * PW:3 * PW]))

        def scores(i):
            sc = _dot(q.pop(i), kk.pop(i), _NT) * b_scale
            sc = jnp.where(mask, sc, MASK_VALUE)
            m0 = jnp.max(jnp.where(first, sc, -jnp.inf), axis=1, keepdims=True)
            m1 = jnp.max(jnp.where(first, -jnp.inf, sc), axis=1, keepdims=True)
            e = jnp.exp(sc - jnp.where(first, m0, m1))
            s0 = jnp.sum(jnp.where(first, e, 0.0), axis=1, keepdims=True)
            s1 = jnp.sum(jnp.where(first, 0.0, e), axis=1, keepdims=True)
            p[i] = e / jnp.where(first, s0, s1)

        def values(i):
            o[i] = _dot(p.pop(i), vv.pop(i))

        def out_proj(i):
            oi = o.pop(i)
            r = _dot(jnp.concatenate([oi[seg:], oi[:seg]], axis=0), wo_v[i * PW:(i + 1) * PW, :])
            acc[0] = r if acc[0] is None else acc[0] + r

        done = 0
        i = 0
        while done < n_pair:
            if i < n_pair:
                project(i)
            if 0 <= i - D_QK < n_pair:
                scores(i - D_QK)
            if 0 <= i - D_PV < n_pair:
                values(i - D_PV)
            if i < n_pair:
                n = 1 if i >= D_WO else 0
            else:
                left = n_pair + D_PV - i
                ready = min(n_pair, i - D_PV) - done
                n = min(-(-(n_pair - 1 - done) // left), ready) if left > 0 else n_pair - done
            for _ in range(n):
                out_proj(done)
                done += 1
            i += 1

        h_v[(slot + 1) % B_UNROLL, seg:L, :] = acc[0][:M]
        rows = pl.ds(pl.multiple_of(s * seg, seg), seg)
        bout_v[rows, :] = acc[0][M:].astype(BF16)
        pltpu.make_async_copy(
            bout_v.at[rows], out_hbm.at[rows, pl.ds(D, D)], sem_out.at[1]).start()

    def b_step(g, carry):
        for slot in range(B_UNROLL):
            b_segment(g, slot)
        return carry

    lax.fori_loop(0, n_seg // B_UNROLL, b_step, 0)

    cp_aout.wait()
    pltpu.make_async_copy(bout_v, out_hbm.at[:, pl.ds(D, D)], sem_out.at[1]).wait()


@functools.partial(jax.jit, static_argnames=("B_seg_len",))
def pallas_concat_heads__sliding_local_dilated__memory_aug_recurrent_mem_tr__prompt_kernel(
    A_x: jax.Array,
    A_wqkv: jax.Array,
    A_wo: jax.Array,
    B_x: jax.Array,
    B_mem0: jax.Array,
    B_Wq: jax.Array,
    B_Wk: jax.Array,
    B_Wv: jax.Array,
    B_Wo: jax.Array,
    B_seg_len: int,
):
    B, S, D = A_x.shape
    M = B_mem0.shape[1]
    _, H, Dh = B_Wq.shape
    seg = int(B_seg_len)
    n_t = D // LANES
    n_seg = S // seg
    n_chunk = S // A_CHUNK
    n_pair = H // 2
    assert B == 1 and B_x.shape == (B, S, D) and S % A_CHUNK == 0 and S % seg == 0
    assert D % LANES == 0 and D % A_HEADS == 0 and 4 * A_HEADS == LANES
    assert 2 * Dh == 3 * LANES and 2 * (seg + M) <= LANES and seg % 16 == 0 and M % 8 == 0
    assert H % 2 == 0 and n_seg % B_UNROLL == 0 and (n_seg * PRE) % PRE_ROWS == 0
    assert n_pair % N_GROUP == 0 and (n_pair - N_FIRST - 3 * N_REGROUP) % N_GROUP == 0

    def head_major(w):
        return jnp.transpose(w, (1, 2, 0)).reshape(H * Dh, D)

    any_spec = pl.BlockSpec(memory_space=pl.ANY)
    out = pl.pallas_call(
        functools.partial(_kernel, seg=seg, b_heads=H, b_dh=Dh),
        in_specs=[any_spec] * 9,
        out_specs=any_spec,
        out_shape=jax.ShapeDtypeStruct((S, 2 * D), BF16),
        scratch_shapes=[
            pltpu.VMEM((S, D), BF16),
            pltpu.VMEM((4, D, D), BF16),
            pltpu.VMEM((4, D // 2, D), U32),
            pltpu.VMEM((n_t, D + A_HEADS, LANES), F32),
            pltpu.VMEM((n_t, A_HALO + A_CHUNK, LANES), F32),
            pltpu.VMEM((n_t, A_HALO + A_CHUNK, LANES), F32),
            pltpu.VMEM((S, D), BF16),
            pltpu.VMEM((n_seg // 2, 2 * seg, D), BF16),
            pltpu.VMEM((M, D), BF16),
            pltpu.VMEM((3, H * Dh, D), BF16),
            pltpu.VMEM((n_pair, D // 2, 6 * Dh), U32),
            pltpu.VMEM((H * Dh, D), BF16),
            pltpu.VMEM((n_seg // 2, 2 * PRE, D), BF16),
            pltpu.VMEM((n_pair, n_seg * PRE, 2 * Dh), F32),
            pltpu.VMEM((B_UNROLL, seg + M, D), F32),
            pltpu.VMEM((S, D), BF16),
            pltpu.SemaphoreType.DMA((5 + N_FIRST + n_chunk + N_GROUP,)),
            pltpu.SemaphoreType.DMA((2,)),
        ],
        compiler_params=pltpu.CompilerParams(vmem_limit_bytes=104 * 1024 * 1024),
        name="fused_local_attn_rmt",
    )(
        A_x.reshape(S, D),
        A_wqkv,
        A_wo,
        B_x.reshape(n_seg // 2, 2 * seg, D),
        B_mem0.reshape(M, D),
        head_major(B_Wq),
        head_major(B_Wk),
        head_major(B_Wv),
        B_Wo.reshape(H * Dh, D),
    )
    return out.reshape(B, S, 2 * D)
```

```python
import functools

import jax
import jax.numpy as jnp
from jax import lax
import jax.experimental.pallas as pl
import jax.experimental.pallas.tpu as pltpu

BF16 = jnp.bfloat16
F32 = jnp.float32
U32 = jnp.uint32
LANES = 128
MASK_VALUE = -1000000000.0

_NN = (((1,), (0,)), ((), ()))
_NT = (((1,), (1,)), ((), ()))

A_HEADS = 32
A_WIN = 8
A_DIL = 2

A_HALO = 16
A_CHUNK = 256
A_ROWS = 64
A_SUB = 8
A_D_OUT = 3

B_UNROLL = 4
D_QK, D_PV, D_WO = 1, 3, 8
PRE = 8
PRE_ROWS = 128
N_FIRST = 2
N_REGROUP = 2
N_GROUP = 2


def _dot(a, b, dims=_NN):
    return lax.dot_general(a, b, dims, preferred_element_type=F32)


def _tile(x, t):
    return x[:, t * LANES:(t + 1) * LANES]


def _kernel(
    ax_hbm, awqkv_hbm, awo_hbm, bx_hbm, mem_hbm, wq_hbm, wk_hbm, wv_hbm, wo_hbm,
    out_hbm,
    ax_v, aw_v, aw_p, atmp_v, ak_v, av_v, aout_v,
    bx_v, mem_v, wt_v, wqkv_v, wo_v, xpre_v, qpre_v, h_v, bout_v,
    sem_in, sem_out,
    *, seg, b_heads, b_dh,
):
    S, D = ax_hbm.shape
    n_t = D // LANES
    a_dh = D // A_HEADS
    n_chunk = S // A_CHUNK
    M = mem_hbm.shape[0]
    L = seg + M
    n_seg = S // seg
    n_pair = b_heads // 2
    PW = 2 * b_dh
    wt_hbm = (wq_hbm, wk_hbm, wv_hbm)

    n_early = N_FIRST + 3 * N_REGROUP
    n_late = (n_pair - n_early) // N_GROUP
    ppg = n_pair // N_GROUP
    S_B, S_AWO, S_FIRST = 0, 1, 2
    S_REGROUP = S_FIRST + N_FIRST
    S_CHUNK = S_REGROUP + 3
    S_GROUP = S_CHUNK + n_chunk

    def pair_rows(i, n=1):
        return pl.ds(pl.multiple_of(i * PW, PW), n * PW)

    def cp_wt(m, rows, sem):
        return pltpu.make_async_copy(wt_hbm[m].at[rows], wt_v.at[m, rows], sem)

    def cp_first(i):
        sem = sem_in.at[S_FIRST + i]
        cps = [cp_wt(0, pair_rows(i), sem)]
        if i == 0:
            cps += [
                pltpu.make_async_copy(
                    bx_hbm.at[:, pl.ds(u * seg, PRE)], xpre_v.at[:, pl.ds(u * PRE, PRE)], sem)
                for u in range(2)]
        return cps

    def cp_regroup(j):
        sem = sem_in.at[S_REGROUP + j]
        cols = pl.ds(pl.multiple_of(j * D, LANES), D)
        return [
            pltpu.make_async_copy(awqkv_hbm.at[:, cols], aw_v.at[j], sem),
            cp_wt(0, pair_rows(N_FIRST + j * N_REGROUP, N_REGROUP), sem),
        ]

    cp_awo = pltpu.make_async_copy(awo_hbm, aw_v.at[3], sem_in.at[S_AWO])

    def cp_chunk(c):
        rows = pl.ds(pl.multiple_of(c * A_CHUNK, A_CHUNK), A_CHUNK)
        return pltpu.make_async_copy(ax_hbm.at[rows], ax_v.at[rows], sem_in.at[S_CHUNK + c])

    def cp_group(g):
        sem = sem_in.at[S_GROUP + g]
        return [
            cp_wt(0, pair_rows(n_early + g * n_late, n_late), sem),
            cp_wt(1, pair_rows(g * ppg, ppg), sem),
            cp_wt(2, pair_rows(g * ppg, ppg), sem),
        ]

    cp_b = [
        pltpu.make_async_copy(wo_hbm, wo_v, sem_in.at[S_B]),
        pltpu.make_async_copy(mem_hbm, mem_v, sem_in.at[S_B]),
        pltpu.make_async_copy(bx_hbm, bx_v, sem_in.at[S_B]),
    ]

    for i in range(N_FIRST):
        for cp in cp_first(i):
            cp.start()
    for j in range(3):
        for cp in cp_regroup(j):
            cp.start()
    cp_awo.start()
    for c in range(n_chunk):
        cp_chunk(c).start()
    for g in range(N_GROUP):
        for cp in cp_group(g):
            cp.start()
    for cp in cp_b:
        cp.start()

    atmp_v[:, D:, :] = jnp.zeros((n_t, atmp_v.shape[1] - D, LANES), F32)

    def regroup_rows(w):
        for t in range(n_t):
            atmp_v[t, 0:D, :] = _tile(w, t)
        return jnp.concatenate([
            jnp.concatenate(
                [atmp_v[t, pl.ds(d, A_HEADS, stride=a_dh), :] for t in range(n_t)], axis=1
            ).astype(BF16)
            for d in range(a_dh)
        ], axis=0)

    def leading_queries(i):
        n = PRE_ROWS // (2 * PRE)
        for b in range(n_seg * PRE // PRE_ROWS):
            x = xpre_v[b * n:(b + 1) * n].reshape(PRE_ROWS, D)
            qpre_v[i, b * PRE_ROWS:(b + 1) * PRE_ROWS, :] = _dot(
                x, wt_v[0, pair_rows(i), :], _NT)

    def transpose_w(i, m):
        wqkv_v[i, :, m * PW:(m + 1) * PW] = pltpu.bitcast(wt_v[m, pair_rows(i), :].T, U32)

    for i in range(N_FIRST):
        for cp in cp_first(i):
            cp.wait()
        leading_queries(i)
        transpose_w(i, 0)

    def regroup(j, carry):
        for cp in cp_regroup(j):
            cp.wait()
        aw_p[j] = pltpu.bitcast(regroup_rows(aw_v[j].astype(F32).T).T, U32)
        for n in range(N_REGROUP):
            leading_queries(N_FIRST + j * N_REGROUP + n)
            transpose_w(N_FIRST + j * N_REGROUP + n, 0)
        return carry

    lax.fori_loop(0, 3, regroup, 0)
    cp_awo.wait()
    aw_p[3] = pltpu.bitcast(regroup_rows(aw_v[3].astype(F32)), U32)

    a_scale = float(a_dh) ** -0.5
    for buf in (ak_v, av_v):
        buf[:, 0:A_HALO, :] = jnp.zeros((n_t, A_HALO, LANES), F32)

    def a_chunk(c, carry):
        r0 = pl.multiple_of(c * A_CHUNK, A_CHUNK)
        cp_chunk(c).wait()
        qs, outs = {}, {}

        def project(i):
            x = ax_v[pl.ds(r0 + i * A_ROWS, A_ROWS), :]
            rows = pl.ds(A_HALO + i * A_ROWS, A_ROWS)
            v = _dot(x, pltpu.bitcast(aw_p[2], BF16))
            for t in range(n_t):
                av_v[t, rows, :] = _tile(v, t)
            if i == 0:
                for t in range(n_t):
                    row0 = jnp.broadcast_to(_tile(v, t)[0:1], (A_HALO, LANES))
                    av_v[t, 0:A_HALO, :] = jnp.where(c == 0, row0, av_v[t, 0:A_HALO, :])
            k = _dot(x, pltpu.bitcast(aw_p[1], BF16))
            for t in range(n_t):
                ak_v[t, rows, :] = _tile(k, t)
            qs[i] = _dot(x, pltpu.bitcast(aw_p[0], BF16))

        def attend(i):
            q = qs.pop(i)
            blocks = []
            for rq in range(0, A_ROWS, A_SUB):
                rb = i * A_ROWS + rq
                window = [pl.ds(A_HALO + rb - w * A_DIL, A_SUB) for w in range(A_WIN)]
                logits = []
                for w, rows in enumerate(window):
                    acc = functools.reduce(jnp.add, [
                        _tile(q, t)[rq:rq + A_SUB] * ak_v[t, rows, :] for t in range(n_t)])
                    acc = acc + pltpu.roll(acc, 2 * A_HEADS, axis=1)
                    acc = acc + pltpu.roll(acc, A_HEADS, axis=1)
                    lg = acc * a_scale
                    if rb < w * A_DIL:
                        pos = r0 + rb + lax.broadcasted_iota(jnp.int32, (A_SUB, LANES), 0)
                        lg = jnp.where(pos >= w * A_DIL, lg, MASK_VALUE)
                    logits.append(lg)
                mx = functools.reduce(jnp.maximum, logits)
                es = [jnp.exp(lg - mx) for lg in logits]
                inv = 1.0 / functools.reduce(jnp.add, es)
                blocks.append(jnp.concatenate([
                    (functools.reduce(
                        jnp.add, [e * av_v[t, rows, :] for e, rows in zip(es, window)]
                    ) * inv).astype(BF16)
                    for t in range(n_t)], axis=1))
            outs[i] = jnp.concatenate(blocks, axis=0)

        def out_proj(i):
            y = _dot(outs.pop(i), pltpu.bitcast(aw_p[3], BF16))
            aout_v[pl.ds(r0 + i * A_ROWS, A_ROWS), :] = y.astype(BF16)

        n_sub = A_CHUNK // A_ROWS
        for i in range(n_sub + A_D_OUT):
            if i < n_sub:
                project(i)
            if 0 <= i - 1 < n_sub:
                attend(i - 1)
            if 0 <= i - A_D_OUT < n_sub:
                out_proj(i - A_D_OUT)
        for buf in (ak_v, av_v):
            buf[:, 0:A_HALO, :] = buf[:, A_CHUNK:A_CHUNK + A_HALO, :]
        return carry

    lax.fori_loop(0, n_chunk, a_chunk, 0)

    cp_aout = pltpu.make_async_copy(aout_v, out_hbm.at[:, pl.ds(0, D)], sem_out.at[0])
    cp_aout.start()

    def prepare_group(g, carry):
        for cp in cp_group(g):
            cp.wait()
        for n in range(n_late):
            leading_queries(n_early + g * n_late + n)
            transpose_w(n_early + g * n_late + n, 0)
        for n in range(ppg):
            transpose_w(g * ppg + n, 1)
            transpose_w(g * ppg + n, 2)
        return carry

    lax.fori_loop(0, N_GROUP, prepare_group, 0)
    for cp in cp_b:
        cp.wait()

    b_scale = float(b_dh) ** -0.5
    h_v[0, seg:L, :] = mem_v[...].astype(F32)

    def b_segment(g, slot):
        s = g * B_UNROLL + slot
        x = bx_v[g * (B_UNROLL // 2) + slot // 2, (slot % 2) * seg:(slot % 2 + 1) * seg, :]
        h_v[slot, 0:seg, :] = x.astype(F32)

        row = lax.broadcasted_iota(jnp.int32, (L, 2 * L), 0)
        col = lax.broadcasted_iota(jnp.int32, (L, 2 * L), 1)
        first = col < L
        key = jnp.where(first, col, col - L)
        mask = (row >= seg) | (key >= seg) | (key <= row)
        lo = lax.broadcasted_iota(jnp.int32, (L, LANES), 1) < b_dh - LANES

        def block_diag(t):
            z = jnp.zeros((L, LANES), F32)
            top = jnp.concatenate([_tile(t, 0), jnp.where(lo, _tile(t, 1), 0.0), z], axis=1)
            bot = jnp.concatenate([z, jnp.where(lo, 0.0, _tile(t, 1)), _tile(t, 2)], axis=1)
            return jnp.concatenate([top, bot], axis=0).astype(BF16)

        q, kk, vv, p, o = {}, {}, {}, {}, {}
        acc = [None]

        def project(i):
            h = h_v[slot]
            w = pltpu.bitcast(wqkv_v[i], BF16)
            if i == 0 and slot > 0:
                for t in range(n_t):
                    wt = w[t * LANES:(t + 1) * LANES]
                    kt = _dot(_tile(h, t), wt[:, PW:2 * PW])
                    qt = _dot(_tile(h[PRE:], t), wt[:, 0:PW])
                    k, q_rest = (kt, qt) if t == 0 else (k + kt, q_rest + qt)
            else:
                k = _dot(h, w[:, PW:2 * PW])
                q_rest = _dot(h[PRE:], w[:, 0:PW])
            v = _dot(h, w[:, 2 * PW:3 * PW])
            kk[i] = block_diag(k)
            q[i] = jnp.concatenate(
                [qpre_v[i, pl.ds(pl.multiple_of(s * PRE, PRE), PRE), :], q_rest], axis=0)
            vv[i] = block_diag(v)

        def scores(i):
            sc = _dot(q.pop(i), kk.pop(i), _NT) * b_scale
            sc = jnp.where(mask, sc, MASK_VALUE)
            m0 = jnp.max(jnp.where(first, sc, -jnp.inf), axis=1, keepdims=True)
            m1 = jnp.max(jnp.where(first, -jnp.inf, sc), axis=1, keepdims=True)
            e = jnp.exp(sc - jnp.where(first, m0, m1))
            s0 = jnp.sum(jnp.where(first, e, 0.0), axis=1, keepdims=True)
            s1 = jnp.sum(jnp.where(first, 0.0, e), axis=1, keepdims=True)
            p[i] = e / jnp.where(first, s0, s1)

        def values(i):
            o[i] = _dot(p.pop(i), vv.pop(i))

        def out_proj(i):
            oi = o.pop(i)
            r = _dot(jnp.concatenate([oi[seg:], oi[:seg]], axis=0), wo_v[i * PW:(i + 1) * PW, :])
            acc[0] = r if acc[0] is None else acc[0] + r

        done = 0
        for i in range(n_pair + D_PV):
            if i < n_pair:
                project(i)
            if 0 <= i - D_QK < n_pair:
                scores(i - D_QK)
            if 0 <= i - D_PV < n_pair:
                values(i - D_PV)
            if i < n_pair:
                n = 1 if i >= D_WO else 0
            else:
                n = min(pl.cdiv(n_pair - 1 - done, n_pair + D_PV - i), i - D_PV - done)
            for _ in range(n):
                out_proj(done)
                done += 1
        for i in range(done, n_pair):
            out_proj(i)

        h_v[(slot + 1) % B_UNROLL, seg:L, :] = acc[0][:M]
        rows = pl.ds(pl.multiple_of(s * seg, seg), seg)
        bout_v[rows, :] = acc[0][M:].astype(BF16)
        pltpu.make_async_copy(
            bout_v.at[rows], out_hbm.at[rows, pl.ds(D, D)], sem_out.at[1]).start()

    def b_step(g, carry):
        for slot in range(B_UNROLL):
            b_segment(g, slot)
        return carry

    lax.fori_loop(0, n_seg // B_UNROLL, b_step, 0)

    cp_aout.wait()
    pltpu.make_async_copy(bout_v, out_hbm.at[:, pl.ds(D, D)], sem_out.at[1]).wait()


@functools.partial(jax.jit, static_argnames=("B_seg_len",))
def pallas_concat_heads__sliding_local_dilated__memory_aug_recurrent_mem_tr__prompt_kernel(
    A_x: jax.Array,
    A_wqkv: jax.Array,
    A_wo: jax.Array,
    B_x: jax.Array,
    B_mem0: jax.Array,
    B_Wq: jax.Array,
    B_Wk: jax.Array,
    B_Wv: jax.Array,
    B_Wo: jax.Array,
    B_seg_len: int,
):
    B, S, D = A_x.shape
    M = B_mem0.shape[1]
    _, H, Dh = B_Wq.shape
    seg = int(B_seg_len)
    n_t = D // LANES
    n_seg = S // seg
    n_chunk = S // A_CHUNK
    n_pair = H // 2
    assert B == 1 and B_x.shape == (B, S, D) and S % A_CHUNK == 0 and S % seg == 0
    assert D % LANES == 0 and D % A_HEADS == 0 and 4 * A_HEADS == LANES
    assert 2 * Dh == 3 * LANES and 2 * (seg + M) <= LANES and seg % 16 == 0 and M % 8 == 0
    assert H % 2 == 0 and n_seg % B_UNROLL == 0 and (n_seg * PRE) % PRE_ROWS == 0
    assert n_pair % N_GROUP == 0 and (n_pair - N_FIRST - 3 * N_REGROUP) % N_GROUP == 0

    def head_major(w):
        return jnp.transpose(w, (1, 2, 0)).reshape(H * Dh, D)

    any_spec = pl.BlockSpec(memory_space=pl.ANY)
    out = pl.pallas_call(
        functools.partial(_kernel, seg=seg, b_heads=H, b_dh=Dh),
        in_specs=[any_spec] * 9,
        out_specs=any_spec,
        out_shape=jax.ShapeDtypeStruct((S, 2 * D), BF16),
        scratch_shapes=[
            pltpu.VMEM((S, D), BF16),
            pltpu.VMEM((4, D, D), BF16),
            pltpu.VMEM((4, D // 2, D), U32),
            pltpu.VMEM((n_t, D + A_HEADS, LANES), F32),
            pltpu.VMEM((n_t, A_HALO + A_CHUNK, LANES), F32),
            pltpu.VMEM((n_t, A_HALO + A_CHUNK, LANES), F32),
            pltpu.VMEM((S, D), BF16),
            pltpu.VMEM((n_seg // 2, 2 * seg, D), BF16),
            pltpu.VMEM((M, D), BF16),
            pltpu.VMEM((3, H * Dh, D), BF16),
            pltpu.VMEM((n_pair, D // 2, 6 * Dh), U32),
            pltpu.VMEM((H * Dh, D), BF16),
            pltpu.VMEM((n_seg // 2, 2 * PRE, D), BF16),
            pltpu.VMEM((n_pair, n_seg * PRE, 2 * Dh), F32),
            pltpu.VMEM((B_UNROLL, seg + M, D), F32),
            pltpu.VMEM((S, D), BF16),
            pltpu.SemaphoreType.DMA((5 + N_FIRST + n_chunk + N_GROUP,)),
            pltpu.SemaphoreType.DMA((2,)),
        ],
        compiler_params=pltpu.CompilerParams(vmem_limit_bytes=104 * 1024 * 1024),
        name="fused_local_attn_rmt",
    )(
        A_x.reshape(S, D),
        A_wqkv,
        A_wo,
        B_x.reshape(n_seg // 2, 2 * seg, D),
        B_mem0.reshape(M, D),
        head_major(B_Wq),
        head_major(B_Wk),
        head_major(B_Wv),
        B_Wo.reshape(H * Dh, D),
    )
    return out.reshape(B, S, 2 * D)
```
